```python
import jax
import jax.numpy as jnp

def _softmax(x, axis=-1):
    return jax.nn.softmax(x, axis=axis)
def _gelu(x):
    return jax.nn.gelu(x, approximate=True)
def _silu(x):
    return jax.nn.silu(x)
def _sigmoid(x):
    return jax.nn.sigmoid(x)
def _layernorm(x, axis=-1, eps=1e-5):
    m = jnp.mean(x, axis=axis, keepdims=True)
    v = jnp.var(x, axis=axis, keepdims=True)
    return (x - m) / jnp.sqrt(v + eps)
def _scatter_add(tgt, idx, src, axis=0):
    return tgt.at[idx].add(src)
def _segment_sum(src, seg, n):
    return jax.ops.segment_sum(src, seg, n)
class _Rng:
    def __init__(self, key):
        self._k = key
    def _next(self):
        self._k, sub = jax.random.split(self._k)
        return sub
    def normal(self, shape):
        return jax.random.normal(self._next(), shape, dtype=jnp.bfloat16)
    def randint(self, lo, hi, shape):
        return jax.random.randint(self._next(), shape, lo, hi, dtype=jnp.int32)
    def uniform(self, shape, lo=0.0, hi=1.0):
        return jax.random.uniform(self._next(), shape, jnp.bfloat16, lo, hi)
    def permutation(self, n):
        return jax.random.permutation(self._next(), n)


kernel_name = 'interleave_layers__sliding_local_dilated__spectral_gfnet__prompt'

def setup_inputs():
    _rng = _Rng(jax.random.key(int.from_bytes(__import__("os").urandom(4), "little")))
    _w = (lambda a: (lambda t: t.astype(jnp.bfloat16) if jnp.issubdtype(t.dtype, jnp.floating) else t)(jnp.asarray(a)))
    def _A_setup():
        B, S, D = 1, 2048, 1024
        return {
            "x": _w((lambda *s: _rng.normal(s) * 0.05)(B, S, D)),
            "wqkv": _w((lambda *s: _rng.normal(s) * 0.05)(D, 3 * D)),
            "wo": _w((lambda *s: _rng.normal(s) * 0.05)(D, D)),
        }
    _A_in = _A_setup()

    def _B_setup():
        B, S, D = 1, 2048, 1024
        Df = D // 2 + 1
        return {
            "x": _w((lambda *s: _rng.normal(s) * 0.05)(B, S, D)),
            "w_r": _w((lambda *s: _rng.normal(s) * 0.05)(S, Df) * 0.02),
            "w_i": _w((lambda *s: _rng.normal(s) * 0.05)(S, Df) * 0.02),
        }
    _B_in = _B_setup()

    return {
        "A_x": _A_in["x"],
        "A_wqkv": _A_in["wqkv"],
        "A_wo": _A_in["wo"],
        "B_x": _B_in["x"],
        "B_w_r": _B_in["w_r"],
        "B_w_i": _B_in["w_i"],
    }

def reference(A_x, A_wqkv, A_wo, B_x, B_w_r, B_w_i):
    def _A_ref(x, wqkv, wo):
        B, S, D = x.shape
        H = 32; Dh = D // H
        W, dil = 8, 2
        qkv = (lambda x, *d: x.transpose(*d))((x @ wqkv).reshape(B, S, 3, H, Dh), 2, 0, 3, 1, 4)
        q, k, v = qkv[0], qkv[1], qkv[2]
        scale = Dh ** -0.5
        pos = jnp.arange(S)
        off = jnp.arange(W) * dil
        idx = pos[:, None] - off[None, :]
        mask = idx >= 0
        idx_c = jnp.where(mask, idx, 0).reshape(-1)
        kg = k[:, :, idx_c, :].reshape(B, H, S, W, Dh)
        vg = v[:, :, idx_c, :].reshape(B, H, S, W, Dh)
        logits = jnp.einsum("bhsd,bhswd->bhsw", q, kg) * scale
        logits = jnp.where(mask[None, None, :, :], logits, -1e9)
        attn = _softmax(logits, axis=-1)
        o = jnp.einsum("bhsw,bhswd->bhsd", attn, vg)
        return (lambda x, *d: x.transpose(*d))(o, 0, 2, 1, 3).reshape(B, S, D) @ wo

    def _B_ref(x, w_r, w_i):
        B, S, D = x.shape
        X = (lambda x, axes=(-2,-1): jnp.fft.rfft2(x.astype(jnp.float32), axes=axes))(x, axes=(-2, -1))
        W = w_r + 1j * w_i
        X = X * W
        y = (lambda x, s, axes=(-2,-1): jnp.fft.irfft2(x, s=s, axes=axes).astype(jnp.bfloat16))(X, (S, D), axes=(-2, -1))
        return y

    x = A_x
    x = x + _A_ref(_layernorm(x, axis=-1), A_wqkv, A_wo)
    x = x + _B_ref(_layernorm(x, axis=-1), B_w_r, B_w_i)
    x = x + _A_ref(_layernorm(x, axis=-1), A_wqkv, A_wo)
    x = x + _B_ref(_layernorm(x, axis=-1), B_w_r, B_w_i)
    return x
```

```python
import numpy as np
import jax
import jax.numpy as jnp
from jax import lax
import jax.experimental.pallas as pl
import jax.experimental.pallas.tpu as pltpu

S, D = 2048, 1024
BS = 512
RC = 32
GA = 4
F32, BF = jnp.float32, jnp.bfloat16


def _consts():
    d = np.arange(512)[:, None]
    k = np.arange(512)[None, :]
    ang = 2 * np.pi * d * k / 1024
    cf = np.zeros((512, 640)); cf[:, :512] = np.cos(ang); cf[:, 512] = (-1.0) ** d[:, 0]
    sf = -np.sin(ang)
    ci = cf.T.copy(); ci[1:512] *= 2
    si = 2 * np.sin(ang).T
    rev = np.zeros((128, 128)); l = np.arange(128); rev[(128 - l) % 128, l] = 1
    grp = (l[:, None] // 4 == l[None, :] // 4) * 1.0
    mf = np.zeros((16, 256, 256)); mi = np.zeros((16, 256, 256))
    for a in range(16):
        t = 2 * np.pi * l[:, None] * (a + 16 * l[None, :]) / 2048
        c, s = np.cos(t), np.sin(t)
        mf[a] = np.block([[c, s], [-s, c]])
        mi[a] = np.block([[c.T, -s.T], [s.T, c.T]])
    return cf, sf, ci, si, rev, grp, mf, mi


def _dot(a, b):
    return jnp.dot(a, b, preferred_element_type=F32)


def _ln(x):
    m = jnp.mean(x, axis=-1, keepdims=True)
    xc = x - m
    v = jnp.mean(xc * xc, axis=-1, keepdims=True)
    return (xc * lax.rsqrt(v + 1e-5)).astype(BF)


def _fft(v, sign):
    n = len(v)
    if n == 1:
        return v
    e, o = _fft(v[0::2], sign), _fft(v[1::2], sign)
    out = [None] * n
    for k in range(n // 2):
        er, ei = e[k]
        r, i = o[k]
        if k == 0:
            out[k], out[k + n // 2] = (er + r, ei + i), (er - r, ei - i)
        elif 4 * k == n:
            if sign > 0:
                out[k], out[k + n // 2] = (er - i, ei + r), (er + i, ei - r)
            else:
                out[k], out[k + n // 2] = (er + i, ei - r), (er - i, ei + r)
        else:
            c = float(np.cos(2 * np.pi * k / n)); s = float(sign * np.sin(2 * np.pi * k / n))
            if 8 * k == n or 8 * k == 3 * n:
                h = abs(c)
                if c > 0 and s > 0: tr, ti = (r - i) * h, (r + i) * h
                elif c > 0: tr, ti = (r + i) * h, (i - r) * h
                elif s > 0: tr, ti = (r + i) * (-h), (r - i) * h
                else: tr, ti = (i - r) * h, (r + i) * (-h)
            else:
                tr, ti = r * c - i * s, r * s + i * c
            out[k], out[k + n // 2] = (er + tr, ei + ti), (er - tr, ei - ti)
    return out


def _swap_lanes(w_ref, c0):
    def body(r, _):
        rows = pl.ds(pl.multiple_of(r * 64, 64), 64)
        t = [pltpu.bitcast(w_ref[rows, c0 + 128 * u:c0 + 128 * (u + 1)], jnp.int32) for u in range(8)]
        lane = lax.broadcasted_iota(jnp.int32, (32, 128), 1)
        for bit in range(3):
            dist = 4 << bit
            lo = (lane & dist) == 0
            for u in range(8):
                if not u & (1 << bit):
                    a, b = t[u], t[u | (1 << bit)]
                    t[u] = jnp.where(lo, a, pltpu.roll(b, dist, 1))
                    t[u | (1 << bit)] = jnp.where(lo, pltpu.roll(a, 128 - dist, 1), b)
        for u in range(8):
            w_ref[rows, c0 + 128 * u:c0 + 128 * (u + 1)] = pltpu.bitcast(t[u], BF)
        return 0
    lax.fori_loop(0, D // 64, body, 0)


def _swap_rows(w_ref):
    def body(c, _):
        cols = pl.ds(pl.multiple_of(c * 128, 128), 128)
        t = [pltpu.bitcast(w_ref[128 * u:128 * (u + 1), cols], jnp.int32) for u in range(8)]
        row = lax.broadcasted_iota(jnp.int32, (64, 128), 0)
        for bit in range(3):
            dist = 2 << bit
            lo = (row & dist) == 0
            for u in range(8):
                if not u & (1 << bit):
                    a, b = t[u], t[u | (1 << bit)]
                    t[u] = jnp.where(lo, a, pltpu.roll(b, dist, 0))
                    t[u | (1 << bit)] = jnp.where(lo, pltpu.roll(a, 64 - dist, 0), b)
        for u in range(8):
            w_ref[128 * u:128 * (u + 1), cols] = pltpu.bitcast(t[u], BF)
        return 0
    lax.fori_loop(0, D // 128, body, 0)


def _kernel(x_hbm, wqkv_hbm, wo_hbm, wr_hbm, wi_hbm,
            cf, sf, ci, si, rev, grp, mf, mi, out_hbm,
            xb, x, wqkv, wo, wr, wi, q, kb, vb, ob, T, sem):
    cps = [pltpu.make_async_copy(s, d, sem.at[i]) for i, (s, d) in enumerate(
        [(wqkv_hbm, wqkv), (x_hbm, xb), (wo_hbm, wo), (wr_hbm, wr), (wi_hbm, wi)])]
    for c in cps:
        c.start()
    cps[0].wait()
    for j in range(3):
        _swap_lanes(wqkv, j * D)
    cps[1].wait()
    cps[2].wait()
    _swap_rows(wo)

    def ldx(rows):
        return jnp.concatenate([x[t, rows, :] for t in range(8)], 1)

    def stx(rows, v):
        for t in range(8):
            x[t, rows, :] = v[:, 128 * t:128 * (t + 1)]

    def layer_a(first):
        kb[0:16, :] = jnp.zeros((16, D), F32)
        vb[0:16, :] = jnp.zeros((16, D), F32)

        def blk(i, _):
            rows = pl.ds(pl.multiple_of(i * BS, BS), BS)
            if first:
                stx(rows, xb[rows, :].astype(F32))
            h = _ln(ldx(rows))
            q[...] = _dot(h, wqkv[:, 0:D]) * (32 ** -0.5)
            kb[16:, :] = _dot(h, wqkv[:, D:2 * D])
            vb[16:, :] = _dot(h, wqkv[:, 2 * D:])

            def chunk(c, _):
                r0 = pl.multiple_of(c * RC, RC)
                win = pl.ds(r0, RC + 16)
                acc = [None] * 8
                for t in range(8):
                    ls = slice(128 * t, 128 * (t + 1))
                    qq = q[pl.ds(r0, RC), ls]
                    kk = kb[win, ls]
                    for w in range(8):
                        p = qq * kk[16 - 2 * w:16 - 2 * w + RC]
                        acc[w] = p if t == 0 else acc[w] + p
                lg = _dot(jnp.concatenate(acc, 0).astype(BF), grp[...])
                pos = i * BS + r0 + lax.broadcasted_iota(jnp.int32, (RC, 128), 0)
                lg = [jnp.where(pos >= 2 * w, lg[w * RC:(w + 1) * RC], -1e9) for w in range(8)]
                m = lg[0]
                for w in range(1, 8):
                    m = jnp.maximum(m, lg[w])
                e = [jnp.exp(l - m) for l in lg]
                tot = e[0]
                for w in range(1, 8):
                    tot = tot + e[w]
                inv = 1.0 / tot
                e = [z * inv for z in e]
                for t in range(8):
                    ls = slice(128 * t, 128 * (t + 1))
                    vv = vb[win, ls]
                    o = e[0] * vv[16:16 + RC]
                    for w in range(1, 8):
                        o = o + e[w] * vv[16 - 2 * w:16 - 2 * w + RC]
                    ob[pl.ds(r0, RC), ls] = o.astype(BF)
                return 0
            lax.fori_loop(0, BS // RC, chunk, 0)
            kb[0:16, :] = kb[BS:BS + 16, :]
            vb[0:16, :] = vb[BS:BS + 16, :]
            stx(rows, ldx(rows) + _dot(ob[...], wo[...]))
            return 0
        lax.fori_loop(0, S // BS, blk, 0)

    def layer_b():
        n = GA * 128
        lane = lax.broadcasted_iota(jnp.int32, (n, 128), 1)
        l0 = lane == 0
        sgn = jnp.where((lane & 1) == 0, 1.0, -1.0).astype(F32)

        def fwd(g, _):
            xs = jnp.concatenate(
                [ldx(pl.ds(g * GA + j, 128, stride=16)) for j in range(GA)], 0)
            z = _ln(xs)
            up = [z[:, 512 + 128 * t:640 + 128 * t] for t in range(4)]
            rv = [_dot(u, rev[...]) for u in up]
            ze, zo = [], []
            for t in range(4):
                r = jnp.where(l0, rv[4 - t] if t else 0.0, rv[3 - t])
                lo = z[:, 128 * t:128 * (t + 1)].astype(F32)
                ze.append((lo + r).astype(BF))
                zo.append((lo - r).astype(BF))
            zre = _dot(jnp.concatenate(ze, 1), cf[...])
            zim = _dot(jnp.concatenate(zo, 1), sf[...])
            ny = up[0][:, 0:1].astype(F32) * sgn
            zre = jnp.concatenate(
                [zre[:, 128 * t:128 * (t + 1)] + ny for t in range(4)]
                + [zre[:, 512:] + jnp.where(l0, ny, 0.0)], 1).astype(BF)
            zim = jnp.concatenate([zim.astype(BF), jnp.zeros((n, 128), BF)], 1)
            for j in range(GA):
                rs = slice(128 * j, 128 * (j + 1))
                T[g * GA + j] = _dot(mf[g * GA + j], jnp.concatenate([zre[rs], zim[rs]], 0))
            return 0
        lax.fori_loop(0, 16 // GA, fwd, 0)

        sc = 1.0 / (S * D)

        def mid(r, _):
            r0 = pl.multiple_of(r * 16, 16)
            for t in range(5):
                ls = slice(128 * t, 128 * (t + 1))
                ws = []
                for k in range(16):
                    rr = pl.ds(r0 + 128 * k, 16)
                    if t < 4:
                        ws.append((wr[rr, ls].astype(F32) * sc, wi[rr, ls].astype(F32) * sc))
                    else:
                        ws.append((wr[rr, 512:513].astype(F32) * sc, wi[rr, 512:513].astype(F32) * sc))
                for hf in range(2):
                    h0 = pl.multiple_of(r0 + 8 * hf, 8)
                    v = [(T[a, pl.ds(h0, 8), ls], T[a, pl.ds(h0 + 128, 8), ls]) for a in range(16)]
                    v = _fft(v, -1)
                    y = []
                    for k in range(16):
                        a, b = ws[k][0][8 * hf:8 * hf + 8], ws[k][1][8 * hf:8 * hf + 8]
                        y.append((v[k][0] * a - v[k][1] * b, v[k][0] * b + v[k][1] * a))
                    y = _fft(y, 1)
                    for a in range(16):
                        T[a, pl.ds(h0, 8), ls] = y[a][0]
                        T[a, pl.ds(h0 + 128, 8), ls] = y[a][1]
            return 0
        lax.fori_loop(0, 8, mid, 0)

        def inv(g, _):
            us = [_dot(mi[g * GA + j], T[g * GA + j].astype(BF)) for j in range(GA)]
            re = jnp.concatenate([u[:128] for u in us], 0)
            im = jnp.concatenate([u[128:, :512] for u in us], 0)
            ye = _dot(re.astype(BF), ci[...])
            yo = _dot(im.astype(BF), si[...])
            s4 = re[:, 0:128] + re[:, 128:256] + re[:, 256:384] + re[:, 384:512]
            s4 = jnp.where(l0, 2.0 * s4 - re[:, 0:128] + re[:, 512:640], 2.0 * s4) * sgn
            y512 = jnp.sum(s4, axis=1, keepdims=True)
            u = (ye + yo).astype(BF)
            rv = [_dot(u[:, 128 * t:128 * (t + 1)], rev[...]) for t in range(4)]
            y = jnp.concatenate(
                [ye - yo] + [jnp.where(l0, rv[4 - t] if t else y512, rv[3 - t]) for t in range(4)], 1)
            for j in range(GA):
                rs = pl.ds(g * GA + j, 128, stride=16)
                stx(rs, ldx(rs) + y[128 * j:128 * (j + 1)])
            return 0
        lax.fori_loop(0, 16 // GA, inv, 0)

    layer_a(True)
    cps[3].wait()
    cps[4].wait()
    layer_b()
    layer_a(False)
    layer_b()

    outs = []
    for i in range(4):
        rows = pl.ds(i * 512, 512)
        xb[rows, :] = ldx(rows).astype(BF)
        c = pltpu.make_async_copy(xb.at[rows], out_hbm.at[rows], sem.at[i])
        c.start()
        outs.append(c)
    for c in outs:
        c.wait()


@jax.jit
def pallas_interleave_layers__sliding_local_dilated__spectral_gfnet__prompt_kernel(
    A_x, A_wqkv, A_wo, B_x, B_w_r, B_w_i):
    consts = [jnp.asarray(c.astype(np.float32).astype(BF)) for c in _consts()]
    anyspec = pl.BlockSpec(memory_space=pl.ANY)
    V = pltpu.VMEM
    out = pl.pallas_call(
        _kernel,
        out_shape=jax.ShapeDtypeStruct((S, D), BF),
        in_specs=[anyspec] * 5 + [pl.BlockSpec(memory_space=V)] * len(consts),
        out_specs=anyspec,
        scratch_shapes=[
            V((S, D), BF), V((8, S, 128), F32), V((D, 3 * D), BF), V((D, D), BF),
            V((S, 513), BF), V((S, 513), BF),
            V((BS, D), F32), V((BS + 16, D), F32), V((BS + 16, D), F32), V((BS, D), BF),
            V((16, 256, 640), F32), pltpu.SemaphoreType.DMA((5,))],
        compiler_params=pltpu.CompilerParams(vmem_limit_bytes=110 * 2 ** 20),
    )(A_x.reshape(S, D), A_wqkv, A_wo, B_w_r, B_w_i, *consts)
    return out.reshape(1, S, D)
```

```python
import numpy as np
import jax
import jax.numpy as jnp
from jax import lax
import jax.experimental.pallas as pl
import jax.experimental.pallas.tpu as pltpu

S, D = 2048, 1024
BS = 512
RC = 64
GA = 4
F32, BF = jnp.float32, jnp.bfloat16


def _consts():
    d = np.arange(512)[:, None]
    k = np.arange(512)[None, :]
    ang = 2 * np.pi * d * k / 1024
    cf = np.zeros((512, 640)); cf[:, :512] = np.cos(ang); cf[:, 512] = (-1.0) ** d[:, 0]
    sf = -np.sin(ang)
    ci = cf.T.copy(); ci[1:512] *= 2
    si = 2 * np.sin(ang).T
    rev = np.zeros((128, 128)); l = np.arange(128); rev[(128 - l) % 128, l] = 1
    grp = (l[:, None] // 4 == l[None, :] // 4) * 1.0
    mf = np.zeros((16, 256, 256)); mi = np.zeros((16, 256, 256))
    for a in range(16):
        t = 2 * np.pi * l[:, None] * (a + 16 * l[None, :]) / 2048
        c, s = np.cos(t), np.sin(t)
        mf[a] = np.block([[c, s], [-s, c]])
        mi[a] = np.block([[c.T, -s.T], [s.T, c.T]])
    return cf, sf, ci, si, rev, grp, mf, mi


def _dot(a, b):
    return jnp.dot(a, b, preferred_element_type=F32)


def _ln(x):
    m = jnp.mean(x, axis=-1, keepdims=True)
    xc = x - m
    v = jnp.mean(xc * xc, axis=-1, keepdims=True)
    return (xc * lax.rsqrt(v + 1e-5)).astype(BF)


def _fft(v, sign):
    n = len(v)
    if n == 1:
        return v
    e, o = _fft(v[0::2], sign), _fft(v[1::2], sign)
    out = [None] * n
    for k in range(n // 2):
        er, ei = e[k]
        r, i = o[k]
        if k == 0:
            out[k], out[k + n // 2] = (er + r, ei + i), (er - r, ei - i)
        elif 4 * k == n:
            if sign > 0:
                out[k], out[k + n // 2] = (er - i, ei + r), (er + i, ei - r)
            else:
                out[k], out[k + n // 2] = (er + i, ei - r), (er - i, ei + r)
        else:
            c = float(np.cos(2 * np.pi * k / n)); s = float(sign * np.sin(2 * np.pi * k / n))
            if 8 * k == n or 8 * k == 3 * n:
                h = abs(c)
                if c > 0 and s > 0: tr, ti = (r - i) * h, (r + i) * h
                elif c > 0: tr, ti = (r + i) * h, (i - r) * h
                elif s > 0: tr, ti = (r + i) * (-h), (r - i) * h
                else: tr, ti = (i - r) * h, (r + i) * (-h)
            else:
                tr, ti = r * c - i * s, r * s + i * c
            out[k], out[k + n // 2] = (er + tr, ei + ti), (er - tr, ei - ti)
    return out


def _swap_lanes(w_ref, c0):
    def body(r, _):
        rows = pl.ds(pl.multiple_of(r * 64, 64), 64)
        t = [pltpu.bitcast(w_ref[rows, c0 + 128 * u:c0 + 128 * (u + 1)], jnp.int32) for u in range(8)]
        lane = lax.broadcasted_iota(jnp.int32, (32, 128), 1)
        for bit in range(3):
            dist = 4 << bit
            lo = (lane & dist) == 0
            for u in range(8):
                if not u & (1 << bit):
                    a, b = t[u], t[u | (1 << bit)]
                    t[u] = jnp.where(lo, a, pltpu.roll(b, dist, 1))
                    t[u | (1 << bit)] = jnp.where(lo, pltpu.roll(a, 128 - dist, 1), b)
        for u in range(8):
            w_ref[rows, c0 + 128 * u:c0 + 128 * (u + 1)] = pltpu.bitcast(t[u], BF)
        return 0
    lax.fori_loop(0, D // 64, body, 0)


def _swap_rows(w_ref):
    def body(c, _):
        cols = pl.ds(pl.multiple_of(c * 128, 128), 128)
        t = [pltpu.bitcast(w_ref[128 * u:128 * (u + 1), cols], jnp.int32) for u in range(8)]
        row = lax.broadcasted_iota(jnp.int32, (64, 128), 0)
        for bit in range(3):
            dist = 2 << bit
            lo = (row & dist) == 0
            for u in range(8):
                if not u & (1 << bit):
                    a, b = t[u], t[u | (1 << bit)]
                    t[u] = jnp.where(lo, a, pltpu.roll(b, dist, 0))
                    t[u | (1 << bit)] = jnp.where(lo, pltpu.roll(a, 64 - dist, 0), b)
        for u in range(8):
            w_ref[128 * u:128 * (u + 1), cols] = pltpu.bitcast(t[u], BF)
        return 0
    lax.fori_loop(0, D // 128, body, 0)


def _kernel(x_hbm, wqkv_hbm, wo_hbm, wr_hbm, wi_hbm,
            cf, sf, ci, si, rev, grp, mf, mi, out_hbm,
            xb, x, wqkv, wo, wr, wi, q, hb, ob, T, sem):
    cps = [pltpu.make_async_copy(s, d, sem.at[i]) for i, (s, d) in enumerate(
        [(wqkv_hbm, wqkv), (x_hbm, xb), (wo_hbm, wo), (wr_hbm, wr), (wi_hbm, wi)])]
    for c in cps:
        c.start()
    cps[0].wait()
    for j in range(3):
        _swap_lanes(wqkv, j * D)
    cps[1].wait()
    cps[2].wait()
    _swap_rows(wo)

    def ldx(rows):
        return jnp.concatenate([x[t, rows, :] for t in range(8)], 1)

    def stx(rows, v):
        for t in range(8):
            x[t, rows, :] = v[:, 128 * t:128 * (t + 1)]

    def cvt(i, _):
        rows = pl.ds(pl.multiple_of(i * 128, 128), 128)
        stx(rows, xb[rows, :].astype(F32))
        return 0
    lax.fori_loop(0, S // 128, cvt, 0)

    def layer_a():
        NC = BS // RC
        CW = 4 * D // NC
        q[0, 1:3, 0:16, :] = jnp.zeros((2, 16, D), F32)

        def step(i, do_q, do_a, do_o):
            cur = (i + 2) % 2
            nxt = 1 - cur
            if do_q:
                hb[...] = _ln(ldx(pl.ds(pl.multiple_of((i + 1) * BS, BS), BS)))
                if do_a:
                    q[nxt, 1:3, 0:16, :] = q[cur, 1:3, BS:BS + 16, :]

            def attn(c, mm):
                r0 = pl.multiple_of(c * RC, RC)
                win = pl.ds(r0, RC + 16)
                acc = [None] * 8
                for t in range(8):
                    ls = slice(128 * t, 128 * (t + 1))
                    qq = q[cur, 0, pl.ds(r0 + 16, RC), ls] * (32 ** -0.5)
                    kk = q[cur, 1, win, ls]
                    for w in range(8):
                        p = qq * kk[16 - 2 * w:16 - 2 * w + RC]
                        acc[w] = p if t == 0 else acc[w] + p
                lg = _dot(jnp.concatenate(acc, 0).astype(BF), grp[...])
                r2 = mm(1)
                pos = i * BS + r0 + lax.broadcasted_iota(jnp.int32, (RC, 128), 0)
                lg = [jnp.where(pos >= 2 * w, lg[w * RC:(w + 1) * RC], -1e9) for w in range(8)]
                m = lg[0]
                for w in range(1, 8):
                    m = jnp.maximum(m, lg[w])
                e = [jnp.exp(l - m) for l in lg]
                tot = e[0]
                for w in range(1, 8):
                    tot = tot + e[w]
                inv = 1.0 / tot
                e = [z * inv for z in e]
                for t in range(8):
                    ls = slice(128 * t, 128 * (t + 1))
                    vv = q[cur, 2, win, ls]
                    o = e[0] * vv[16:16 + RC]
                    for w in range(1, 8):
                        o = o + e[w] * vv[16 - 2 * w:16 - 2 * w + RC]
                    ob[cur, pl.ds(r0, RC), ls] = o.astype(BF)

                return r2

            HW = CW // 2

            def both(c, ca, do, mm):
                if not do:
                    return attn(ca, lambda j: None)
                r1 = mm(0)
                r2 = attn(ca, mm) if do_a else mm(1)
                return jnp.concatenate([r1, r2], 1)

            def c1(c, _):
                r = both(c, c, do_q, lambda j: _dot(hb[...], wqkv[:, pl.ds(pl.multiple_of(c * CW + j * HW, HW), HW)]))
                if do_q:
                    q[nxt, c // (D // CW), 16:, pl.ds(pl.multiple_of(c % (D // CW) * CW, CW), CW)] = r
                return 0

            def c2(c, _):
                r = both(c, c + 3 * NC // 4, do_o, lambda j: _dot(ob[nxt], wo[:, pl.ds(pl.multiple_of(c * CW + j * HW, HW), HW)]))
                if do_o:
                    rows = pl.ds(pl.multiple_of((i - 1) * BS, BS), BS)
                    for t in range(CW // 128):
                        tt = c * (CW // 128) + t
                        x[tt, rows, :] = x[tt, rows, :] + r[:, 128 * t:128 * (t + 1)]
                return 0
            if do_q or do_a:
                lax.fori_loop(0, 3 * NC // 4, c1, 0)
            if do_o or do_a:
                lax.fori_loop(0, NC // 4, c2, 0)
            return 0
        nb = S // BS
        step(-1, True, False, False)
        step(0, True, True, False)
        lax.fori_loop(1, nb - 1, lambda i, _: step(i, True, True, True), 0)
        step(nb - 1, False, True, True)
        step(nb, False, False, True)

    def layer_b():
        n = GA * 128
        lane = lax.broadcasted_iota(jnp.int32, (n, 128), 1)
        l0 = lane == 0
        sgn = jnp.where((lane & 1) == 0, 1.0, -1.0).astype(F32)

        def fwd(g, _):
            xs = jnp.concatenate(
                [ldx(pl.ds(g * GA + j, 128, stride=16)) for j in range(GA)], 0)
            z = _ln(xs)
            up = [z[:, 512 + 128 * t:640 + 128 * t] for t in range(4)]
            rv = [_dot(u, rev[...]) for u in up]
            ze, zo = [], []
            for t in range(4):
                r = jnp.where(l0, rv[4 - t] if t else 0.0, rv[3 - t])
                lo = z[:, 128 * t:128 * (t + 1)].astype(F32)
                ze.append((lo + r).astype(BF))
                zo.append((lo - r).astype(BF))
            zre = _dot(jnp.concatenate(ze, 1), cf[...])
            zim = _dot(jnp.concatenate(zo, 1), sf[...])
            ny = up[0][:, 0:1].astype(F32) * sgn
            zre = jnp.concatenate(
                [zre[:, 128 * t:128 * (t + 1)] + ny for t in range(4)]
                + [zre[:, 512:] + jnp.where(l0, ny, 0.0)], 1).astype(BF)
            zim = jnp.concatenate([zim.astype(BF), jnp.zeros((n, 128), BF)], 1)
            for j in range(GA):
                rs = slice(128 * j, 128 * (j + 1))
                T[g * GA + j] = _dot(mf[g * GA + j], jnp.concatenate([zre[rs], zim[rs]], 0))
            return 0
        lax.fori_loop(0, 16 // GA, fwd, 0)

        sc = 1.0 / (S * D)

        def mid(r, _):
            r0 = pl.multiple_of(r * 16, 16)
            for t in range(5):
                ls = slice(128 * t, 128 * (t + 1))
                ws = []
                for k in range(16):
                    rr = pl.ds(r0 + 128 * k, 16)
                    if t < 4:
                        ws.append((wr[rr, ls].astype(F32) * sc, wi[rr, ls].astype(F32) * sc))
                    else:
                        ws.append((wr[rr, 512:513].astype(F32) * sc, wi[rr, 512:513].astype(F32) * sc))
                for hf in range(2):
                    h0 = pl.multiple_of(r0 + 8 * hf, 8)
                    v = [(T[a, pl.ds(h0, 8), ls], T[a, pl.ds(h0 + 128, 8), ls]) for a in range(16)]
                    v = _fft(v, -1)
                    y = []
                    for k in range(16):
                        a, b = ws[k][0][8 * hf:8 * hf + 8], ws[k][1][8 * hf:8 * hf + 8]
                        y.append((v[k][0] * a - v[k][1] * b, v[k][0] * b + v[k][1] * a))
                    y = _fft(y, 1)
                    for a in range(16):
                        T[a, pl.ds(h0, 8), ls] = y[a][0]
                        T[a, pl.ds(h0 + 128, 8), ls] = y[a][1]
            return 0
        lax.fori_loop(0, 8, mid, 0)

        def inv(g, _):
            us = [_dot(mi[g * GA + j], T[g * GA + j].astype(BF)) for j in range(GA)]
            re = jnp.concatenate([u[:128] for u in us], 0)
            im = jnp.concatenate([u[128:, :512] for u in us], 0)
            ye = _dot(re.astype(BF), ci[...])
            yo = _dot(im.astype(BF), si[...])
            s4 = re[:, 0:128] + re[:, 128:256] + re[:, 256:384] + re[:, 384:512]
            s4 = jnp.where(l0, 2.0 * s4 - re[:, 0:128] + re[:, 512:640], 2.0 * s4) * sgn
            y512 = jnp.sum(s4, axis=1, keepdims=True)
            u = (ye + yo).astype(BF)
            rv = [_dot(u[:, 128 * t:128 * (t + 1)], rev[...]) for t in range(4)]
            y = jnp.concatenate(
                [ye - yo] + [jnp.where(l0, rv[4 - t] if t else y512, rv[3 - t]) for t in range(4)], 1)
            for j in range(GA):
                rs = pl.ds(g * GA + j, 128, stride=16)
                stx(rs, ldx(rs) + y[128 * j:128 * (j + 1)])
            return 0
        lax.fori_loop(0, 16 // GA, inv, 0)

    cps[3].wait()
    cps[4].wait()

    def pair(_, c):
        layer_a()
        layer_b()
        return c
    lax.fori_loop(0, 2, pair, 0)

    outs = []
    for i in range(4):
        rows = pl.ds(i * 512, 512)
        xb[rows, :] = ldx(rows).astype(BF)
        c = pltpu.make_async_copy(xb.at[rows], out_hbm.at[rows], sem.at[i])
        c.start()
        outs.append(c)
    for c in outs:
        c.wait()


@jax.jit
def pallas_interleave_layers__sliding_local_dilated__spectral_gfnet__prompt_kernel(
    A_x, A_wqkv, A_wo, B_x, B_w_r, B_w_i):
    consts = [jnp.asarray(c.astype(np.float32).astype(BF)) for c in _consts()]
    anyspec = pl.BlockSpec(memory_space=pl.ANY)
    V = pltpu.VMEM
    out = pl.pallas_call(
        _kernel,
        out_shape=jax.ShapeDtypeStruct((S, D), BF),
        in_specs=[anyspec] * 5 + [pl.BlockSpec(memory_space=V)] * len(consts),
        out_specs=anyspec,
        scratch_shapes=[
            V((S, D), BF), V((8, S, 128), F32), V((D, 3 * D), BF), V((D, D), BF),
            V((S, 513), BF), V((S, 513), BF),
            V((2, 3, BS + 16, D), F32), V((BS, D), BF), V((2, BS, D), BF),
            V((16, 256, 640), F32), pltpu.SemaphoreType.DMA((5,))],
        compiler_params=pltpu.CompilerParams(vmem_limit_bytes=110 * 2 ** 20),
    )(A_x.reshape(S, D), A_wqkv, A_wo, B_w_r, B_w_i, *consts)
    return out.reshape(1, S, D)
```

```python
import numpy as np
import jax
import jax.numpy as jnp
from jax import lax
import jax.experimental.pallas as pl
import jax.experimental.pallas.tpu as pltpu

S, D = 2048, 1024
BS = 256
RC = 64
GA = 4
F32, BF = jnp.float32, jnp.bfloat16


def _consts():
    d = np.arange(512)[:, None]
    k = np.arange(512)[None, :]
    ang = 2 * np.pi * d * k / 1024
    cf = np.zeros((512, 640)); cf[:, :512] = np.cos(ang); cf[:, 512] = (-1.0) ** d[:, 0]
    sf = -np.sin(ang)
    ci = cf.T.copy(); ci[1:512] *= 2
    si = 2 * np.sin(ang).T
    rev = np.zeros((128, 128)); l = np.arange(128); rev[(128 - l) % 128, l] = 1
    grp = (l[:, None] // 4 == l[None, :] // 4) * 1.0
    mf = np.zeros((16, 256, 256)); mi = np.zeros((16, 256, 256))
    for a in range(16):
        t = 2 * np.pi * l[:, None] * (a + 16 * l[None, :]) / 2048
        c, s = np.cos(t), np.sin(t)
        mf[a] = np.block([[c, s], [-s, c]])
        mi[a] = np.block([[c.T, -s.T], [s.T, c.T]])
    return cf, sf, ci, si, rev, grp, mf, mi


def _dot(a, b):
    return jnp.dot(a, b, preferred_element_type=F32)


def _ln(x):
    m = jnp.mean(x, axis=-1, keepdims=True)
    xc = x - m
    v = jnp.mean(xc * xc, axis=-1, keepdims=True)
    return (xc * lax.rsqrt(v + 1e-5)).astype(BF)


def _fft(v, sign):
    n = len(v)
    if n == 1:
        return v
    e, o = _fft(v[0::2], sign), _fft(v[1::2], sign)
    out = [None] * n
    for k in range(n // 2):
        er, ei = e[k]
        r, i = o[k]
        if k == 0:
            out[k], out[k + n // 2] = (er + r, ei + i), (er - r, ei - i)
        elif 4 * k == n:
            if sign > 0:
                out[k], out[k + n // 2] = (er - i, ei + r), (er + i, ei - r)
            else:
                out[k], out[k + n // 2] = (er + i, ei - r), (er - i, ei + r)
        else:
            c = float(np.cos(2 * np.pi * k / n)); s = float(sign * np.sin(2 * np.pi * k / n))
            if 8 * k == n or 8 * k == 3 * n:
                h = abs(c)
                if c > 0 and s > 0: tr, ti = (r - i) * h, (r + i) * h
                elif c > 0: tr, ti = (r + i) * h, (i - r) * h
                elif s > 0: tr, ti = (r + i) * (-h), (r - i) * h
                else: tr, ti = (i - r) * h, (r + i) * (-h)
            else:
                tr, ti = r * c - i * s, r * s + i * c
            out[k], out[k + n // 2] = (er + tr, ei + ti), (er - tr, ei - ti)
    return out


def _swap_lanes(w_ref, c0):
    def body(r, _):
        rows = pl.ds(pl.multiple_of(r * 64, 64), 64)
        t = [pltpu.bitcast(w_ref[rows, c0 + 128 * u:c0 + 128 * (u + 1)], jnp.int32) for u in range(8)]
        lane = lax.broadcasted_iota(jnp.int32, (32, 128), 1)
        for bit in range(3):
            dist = 4 << bit
            lo = (lane & dist) == 0
            for u in range(8):
                if not u & (1 << bit):
                    a, b = t[u], t[u | (1 << bit)]
                    t[u] = jnp.where(lo, a, pltpu.roll(b, dist, 1))
                    t[u | (1 << bit)] = jnp.where(lo, pltpu.roll(a, 128 - dist, 1), b)
        for u in range(8):
            w_ref[rows, c0 + 128 * u:c0 + 128 * (u + 1)] = pltpu.bitcast(t[u], BF)
        return 0
    lax.fori_loop(0, D // 64, body, 0)


def _swap_rows(w_ref):
    def body(c, _):
        cols = pl.ds(pl.multiple_of(c * 128, 128), 128)
        t = [pltpu.bitcast(w_ref[128 * u:128 * (u + 1), cols], jnp.int32) for u in range(8)]
        row = lax.broadcasted_iota(jnp.int32, (64, 128), 0)
        for bit in range(3):
            dist = 2 << bit
            lo = (row & dist) == 0
            for u in range(8):
                if not u & (1 << bit):
                    a, b = t[u], t[u | (1 << bit)]
                    t[u] = jnp.where(lo, a, pltpu.roll(b, dist, 0))
                    t[u | (1 << bit)] = jnp.where(lo, pltpu.roll(a, 64 - dist, 0), b)
        for u in range(8):
            w_ref[128 * u:128 * (u + 1), cols] = pltpu.bitcast(t[u], BF)
        return 0
    lax.fori_loop(0, D // 128, body, 0)


def _kernel(x_hbm, wqkv_hbm, wo_hbm, wr_hbm, wi_hbm,
            cf_h, sf_h, ci_h, si_h, rev, grp, mf_h, mi_h, out_hbm,
            xb, x, wqkv, wo, wr, wi, q, hb, ob, T, sem, wrt, wit, cf, sf, ci, si, mf, mi):
    cps = [pltpu.make_async_copy(s, d, sem.at[i]) for i, (s, d) in enumerate(
        [(wqkv_hbm, wqkv), (x_hbm, xb), (wo_hbm, wo), (wr_hbm, wrt), (wi_hbm, wit),
         (cf_h, cf), (sf_h, sf), (ci_h, ci), (si_h, si), (mf_h, mf), (mi_h, mi)])]
    for c in cps[:3]:
        c.start()
    cps[0].wait()
    for j in range(3):
        _swap_lanes(wqkv, j * D)
    cps[1].wait()
    cps[2].wait()
    for c in cps[3:]:
        c.start()
    _swap_rows(wo)

    def ldx(rows):
        return jnp.concatenate([x[t, rows, :] for t in range(8)], 1)

    def stx(rows, v):
        for t in range(8):
            x[t, rows, :] = v[:, 128 * t:128 * (t + 1)]

    def cvt(i, _):
        rows = pl.ds(pl.multiple_of(i * 128, 128), 128)
        stx(rows, xb[rows, :].astype(F32))
        return 0
    lax.fori_loop(0, S // 128, cvt, 0)

    def layer_a():
        NC = BS // RC
        CW = 4 * D // NC
        q[0, 1:3, 0:16, :] = jnp.zeros((2, 16, D), F32)

        def step(i, do_q, do_a, do_o):
            cur = (i + 2) % 2
            nxt = 1 - cur
            if do_q:
                hb[...] = _ln(ldx(pl.ds(pl.multiple_of((i + 1) * BS, BS), BS)))
                if do_a:
                    q[nxt, 1:3, 0:16, :] = q[cur, 1:3, BS:BS + 16, :]

            def attn(c, mm):
                r0 = pl.multiple_of(c * RC, RC)
                win = pl.ds(r0, RC + 16)
                r2 = []
                acc = [None] * 8
                for t in range(8):
                    ls = slice(128 * t, 128 * (t + 1))
                    if t % 4 == 0:
                        r2.append(mm(t // 4))
                    qq = q[cur, 0, pl.ds(r0 + 16, RC), ls] * (32 ** -0.5)
                    kk = q[cur, 1, win, ls]
                    for w in range(8):
                        p = qq * kk[16 - 2 * w:16 - 2 * w + RC]
                        acc[w] = p if t == 0 else acc[w] + p
                lg = _dot(jnp.concatenate(acc, 0).astype(BF), grp[...])
                pos = i * BS + r0 + lax.broadcasted_iota(jnp.int32, (RC, 128), 0)
                lg = [jnp.where(pos >= 2 * w, lg[w * RC:(w + 1) * RC], -1e9) for w in range(8)]
                m = lg[0]
                for w in range(1, 8):
                    m = jnp.maximum(m, lg[w])
                e = [jnp.exp(l - m) for l in lg]
                tot = e[0]
                for w in range(1, 8):
                    tot = tot + e[w]
                inv = 1.0 / tot
                e = [z * inv for z in e]
                for t in range(8):
                    ls = slice(128 * t, 128 * (t + 1))
                    if t % 4 == 0:
                        r2.append(mm(2 + t // 4))
                    vv = q[cur, 2, win, ls]
                    o = e[0] * vv[16:16 + RC]
                    for w in range(1, 8):
                        o = o + e[w] * vv[16 - 2 * w:16 - 2 * w + RC]
                    ob[cur, pl.ds(r0, RC), ls] = o.astype(BF)

                return r2

            HW = CW // 4

            def both(c, ca, do, mm):
                if not do:
                    return attn(ca, lambda j: None)
                return jnp.concatenate(attn(ca, mm) if do_a else [mm(j) for j in range(4)], 1)

            def c1(c, _):
                r = both(c, c, do_q, lambda j: _dot(hb[...], wqkv[:, pl.ds(pl.multiple_of(c * CW + j * HW, HW), HW)]))
                if do_q:
                    q[nxt, c // (D // CW), 16:, pl.ds(pl.multiple_of(c % (D // CW) * CW, CW), CW)] = r
                return 0

            def c2(c, _):
                r = both(c, c + 3 * NC // 4, do_o, lambda j: _dot(ob[nxt], wo[:, pl.ds(pl.multiple_of(c * CW + j * HW, HW), HW)]))
                if do_o:
                    rows = pl.ds(pl.multiple_of((i - 1) * BS, BS), BS)
                    for t in range(CW // 128):
                        tt = c * (CW // 128) + t
                        x[tt, rows, :] = x[tt, rows, :] + r[:, 128 * t:128 * (t + 1)]
                return 0
            if do_q or do_a:
                lax.fori_loop(0, 3 * NC // 4, c1, 0)
            if do_o or do_a:
                lax.fori_loop(0, NC // 4, c2, 0)
            return 0
        nb = S // BS
        step(-1, True, False, False)
        step(0, True, True, False)
        lax.fori_loop(1, nb - 1, lambda i, _: step(i, True, True, True), 0)
        step(nb - 1, False, True, True)
        step(nb, False, False, True)

    def layer_b():
        n = GA * 128
        lane = lax.broadcasted_iota(jnp.int32, (n, 128), 1)
        l0 = lane == 0
        sgn = jnp.where((lane & 1) == 0, 1.0, -1.0).astype(F32)

        def fwd(g, _):
            xs = jnp.concatenate(
                [ldx(pl.ds(g * GA + j, 128, stride=16)) for j in range(GA)], 0)
            z = _ln(xs)
            up = [z[:, 512 + 128 * t:640 + 128 * t] for t in range(4)]
            rv = [_dot(u, rev[...]) for u in up]
            ze, zo = [], []
            for t in range(4):
                r = jnp.where(l0, rv[4 - t] if t else 0.0, rv[3 - t])
                lo = z[:, 128 * t:128 * (t + 1)].astype(F32)
                ze.append((lo + r).astype(BF))
                zo.append((lo - r).astype(BF))
            zre = _dot(jnp.concatenate(ze, 1), cf[...])
            zim = _dot(jnp.concatenate(zo, 1), sf[...])
            ny = up[0][:, 0:1].astype(F32) * sgn
            zre = jnp.concatenate(
                [zre[:, 128 * t:128 * (t + 1)] + ny for t in range(4)]
                + [zre[:, 512:] + jnp.where(l0, ny, 0.0)], 1).astype(BF)
            zim = jnp.concatenate([zim.astype(BF), jnp.zeros((n, 128), BF)], 1)
            for j in range(GA):
                rs = slice(128 * j, 128 * (j + 1))
                T[g * GA + j] = _dot(mf[g * GA + j], jnp.concatenate([zre[rs], zim[rs]], 0))
            return 0
        lax.fori_loop(0, 16 // GA, fwd, 0)

        sc = 1.0 / (S * D)

        def mid(r, _):
            r0 = pl.multiple_of(r * 16, 16)
            for t in range(5):
                ls = slice(128 * t, 128 * (t + 1))
                ws = []
                for k in range(16):
                    rr = pl.ds(r0 + 128 * k, 16)
                    if True:
                        ws.append((wr[rr, ls].astype(F32) * sc, wi[rr, ls].astype(F32) * sc))
                for hf in range(2):
                    h0 = pl.multiple_of(r0 + 8 * hf, 8)
                    v = [(T[a, pl.ds(h0, 8), ls], T[a, pl.ds(h0 + 128, 8), ls]) for a in range(16)]
                    v = _fft(v, -1)
                    y = []
                    for k in range(16):
                        a, b = ws[k][0][8 * hf:8 * hf + 8], ws[k][1][8 * hf:8 * hf + 8]
                        y.append((v[k][0] * a - v[k][1] * b, v[k][0] * b + v[k][1] * a))
                    y = _fft(y, 1)
                    for a in range(16):
                        T[a, pl.ds(h0, 8), ls] = y[a][0]
                        T[a, pl.ds(h0 + 128, 8), ls] = y[a][1]
            return 0
        lax.fori_loop(0, 8, mid, 0)

        def inv(g, _):
            us = [_dot(mi[g * GA + j], T[g * GA + j].astype(BF)) for j in range(GA)]
            re = jnp.concatenate([u[:128] for u in us], 0)
            im = jnp.concatenate([u[128:, :512] for u in us], 0)
            ye = _dot(re.astype(BF), ci[...])
            yo = _dot(im.astype(BF), si[...])
            s4 = re[:, 0:128] + re[:, 128:256] + re[:, 256:384] + re[:, 384:512]
            s4 = jnp.where(l0, 2.0 * s4 - re[:, 0:128] + re[:, 512:640], 2.0 * s4) * sgn
            y512 = jnp.sum(s4, axis=1, keepdims=True)
            u = (ye + yo).astype(BF)
            rv = [_dot(u[:, 128 * t:128 * (t + 1)], rev[...]) for t in range(4)]
            y = jnp.concatenate(
                [ye - yo] + [jnp.where(l0, rv[4 - t] if t else y512, rv[3 - t]) for t in range(4)], 1)
            for j in range(GA):
                rs = pl.ds(g * GA + j, 128, stride=16)
                stx(rs, ldx(rs) + y[128 * j:128 * (j + 1)])
            return 0
        lax.fori_loop(0, 16 // GA, inv, 0)


    def pair(p, c):
        layer_a()

        @pl.when(p == 0)
        def _():
            for cp in cps[3:]:
                cp.wait()

            def tr(j, _):
                rs = pl.ds(pl.multiple_of(j * 256, 256), 256)
                for src, dst in ((wrt, wr), (wit, wi)):
                    dst[rs, 0:512] = src[0:512, rs].T
                    dst[rs, 512:640] = jnp.broadcast_to(
                        src[512:513, rs].astype(F32), (128, 256)).T.astype(BF)
                return 0
            lax.fori_loop(0, S // 256, tr, 0)
        layer_b()
        return c
    lax.fori_loop(0, 2, pair, 0)

    outs = []
    for i in range(4):
        rows = pl.ds(i * 512, 512)
        xb[rows, :] = ldx(rows).astype(BF)
        c = pltpu.make_async_copy(xb.at[rows], out_hbm.at[rows], sem.at[i])
        c.start()
        outs.append(c)
    for c in outs:
        c.wait()


@jax.jit
def pallas_interleave_layers__sliding_local_dilated__spectral_gfnet__prompt_kernel(
    A_x, A_wqkv, A_wo, B_x, B_w_r, B_w_i):
    consts = [jnp.asarray(c.astype(np.float32).astype(BF)) for c in _consts()]
    anyspec = pl.BlockSpec(memory_space=pl.ANY)
    V = pltpu.VMEM
    out = pl.pallas_call(
        _kernel,
        out_shape=jax.ShapeDtypeStruct((S, D), BF),
        in_specs=[anyspec] * 9 + [pl.BlockSpec(memory_space=V)] * 2 + [anyspec] * 2,
        out_specs=anyspec,
        scratch_shapes=[
            V((S, D), BF), V((8, S, 128), F32), V((D, 3 * D), BF), V((D, D), BF),
            V((S, 640), BF), V((S, 640), BF),
            V((2, 3, BS + 16, D), F32), V((BS, D), BF), V((2, BS, D), BF),
            V((16, 256, 640), F32), pltpu.SemaphoreType.DMA((11,)),
            V((513, S), BF), V((513, S), BF)]
        + [V(consts[i].shape, BF) for i in (0, 1, 2, 3, 6, 7)],
        compiler_params=pltpu.CompilerParams(vmem_limit_bytes=110 * 2 ** 20),
    )(A_x.reshape(S, D), A_wqkv, A_wo, B_w_r.T, B_w_i.T, *consts)
    return out.reshape(1, S, D)
```

```python
import numpy as np
import jax
import jax.numpy as jnp
from jax import lax
import jax.experimental.pallas as pl
import jax.experimental.pallas.tpu as pltpu

S, D = 2048, 1024
BS = 256
RC = 64
GA = 4
F32, BF = jnp.float32, jnp.bfloat16


PAIRS = ((0, 4), (1, 7), (2, 6), (3, 5))


def _pack(m):
    u = m.astype(np.float32).astype(BF).view(np.uint16).astype(np.uint32)
    return (u[..., 0::2, :] | (u[..., 1::2, :] << 16)).view(np.int32)


def _consts():
    l = np.arange(128)
    b, j = l[:, None], np.arange(64)[None, :]
    df = np.zeros((4, 256, 256)); di = np.zeros((4, 256, 256))
    for p, (ka, kb) in enumerate(PAIRS):
        ta, tb = (2 * np.pi * b * (k + 8 * j) / 1024 for k in (ka, kb))
        ca, sa, cb, sb = np.cos(ta), np.sin(ta), np.cos(tb), np.sin(tb)
        if p == 0:
            sa[:, 0] = -(-1.0) ** l
            df[p] = np.block([[ca, 0 * ca, -sa, 0 * ca], [0 * ca, cb, 0 * ca, -sb]])
        else:
            df[p] = np.block([[ca, cb, -sa, -sb], [sa, -sb, ca, -cb]])
        di[p] = 2 * df[p].T
    di[0, [0, 128]] /= 2
    grp = (l[:, None] // 4 == l[None, :] // 4) * 1.0
    mf = np.zeros((16, 256, 256)); mi = np.zeros((16, 256, 256))
    for a in range(16):
        t = 2 * np.pi * l[:, None] * (a + 16 * l[None, :]) / 2048
        c, s = np.cos(t), np.sin(t)
        mf[a] = np.block([[c, s], [-s, c]])
        mi[a] = np.block([[c.T, -s.T], [s.T, c.T]]) / (S * D)
    t = 2 * np.pi * l[:, None] * l[None, :] / 128
    f128 = np.concatenate([np.cos(t), -np.sin(t)], 1)
    i128 = f128.T / (S * D)
    r = np.arange(32)
    t = 2 * np.pi * (r[:, None] % 16) * l[None, :] / 2048
    tw = np.concatenate([np.cos(t), -np.sin(t)], 0).astype(np.float32)
    t = 2 * np.pi * (r[:, None] % 16) * (r[None, :] % 16) / 16
    same = r[:, None] // 16 == r[None, :] // 16
    c, s = np.cos(t) * same, np.sin(t) * same
    f16 = np.block([[c, s], [-s, c]])
    return (_pack(np.concatenate([df, di, mf, mi], 0)), _pack(grp), _pack(f128), _pack(i128),
            _pack(np.concatenate([f16, f16.T], 0)), tw)


def _bf(v):
    return pltpu.bitcast(v, BF)


def _i32(v):
    return pltpu.bitcast(v.astype(BF), jnp.int32)


def _dot(a, b):
    return jnp.dot(a, b, preferred_element_type=F32)


def _ln(x):
    m = jnp.mean(x, axis=-1, keepdims=True)
    xc = x - m
    v = jnp.mean(xc * xc, axis=-1, keepdims=True)
    return xc * lax.rsqrt(v + 1e-5)


def _fft(v, sign):
    n = len(v)
    if n == 1:
        return v
    e, o = _fft(v[0::2], sign), _fft(v[1::2], sign)
    out = [None] * n
    for k in range(n // 2):
        er, ei = e[k]
        r, i = o[k]
        if k == 0:
            out[k], out[k + n // 2] = (er + r, ei + i), (er - r, ei - i)
        elif 4 * k == n:
            if sign > 0:
                out[k], out[k + n // 2] = (er - i, ei + r), (er + i, ei - r)
            else:
                out[k], out[k + n // 2] = (er + i, ei - r), (er - i, ei + r)
        else:
            c = float(np.cos(2 * np.pi * k / n)); s = float(sign * np.sin(2 * np.pi * k / n))
            if 8 * k == n or 8 * k == 3 * n:
                h = abs(c)
                if c > 0 and s > 0: tr, ti = (r - i) * h, (r + i) * h
                elif c > 0: tr, ti = (r + i) * h, (i - r) * h
                elif s > 0: tr, ti = (r + i) * (-h), (r - i) * h
                else: tr, ti = (i - r) * h, (r + i) * (-h)
            else:
                tr, ti = r * c - i * s, r * s + i * c
            out[k], out[k + n // 2] = (er + tr, ei + ti), (er - tr, ei - ti)
    return out


def _swap_lanes(w_ref, o_ref, c0):
    def body(r, _):
        rows = pl.ds(pl.multiple_of(r * 64, 64), 64)
        t = [pltpu.bitcast(w_ref[rows, c0 + 128 * u:c0 + 128 * (u + 1)], jnp.int32) for u in range(8)]
        lane = lax.broadcasted_iota(jnp.int32, (32, 128), 1)
        for bit in range(3):
            dist = 4 << bit
            lo = (lane & dist) == 0
            for u in range(8):
                if not u & (1 << bit):
                    a, b = t[u], t[u | (1 << bit)]
                    t[u] = jnp.where(lo, a, pltpu.roll(b, dist, 1))
                    t[u | (1 << bit)] = jnp.where(lo, pltpu.roll(a, 128 - dist, 1), b)
        for u in range(8):
            o_ref[pl.ds(pl.multiple_of(r * 32, 32), 32), c0 + 128 * u:c0 + 128 * (u + 1)] = t[u]
        return 0
    lax.fori_loop(0, D // 64, body, 0)


def _swap_rows(w_ref, o_ref):
    def body(c, _):
        cols = pl.ds(pl.multiple_of(c * 128, 128), 128)
        t = [pltpu.bitcast(w_ref[128 * u:128 * (u + 1), cols], jnp.int32) for u in range(8)]
        row = lax.broadcasted_iota(jnp.int32, (64, 128), 0)
        for bit in range(3):
            dist = 2 << bit
            lo = (row & dist) == 0
            for u in range(8):
                if not u & (1 << bit):
                    a, b = t[u], t[u | (1 << bit)]
                    t[u] = jnp.where(lo, a, pltpu.roll(b, dist, 0))
                    t[u | (1 << bit)] = jnp.where(lo, pltpu.roll(a, 64 - dist, 0), b)
        for u in range(8):
            o_ref[64 * u:64 * (u + 1), cols] = t[u]
        return 0
    lax.fori_loop(0, D // 128, body, 0)


def _kernel(x_hbm, wqkv_hbm, wo_hbm, wr_hbm, wi_hbm, cm_hbm, grp, f128, i128, f16, tw, out_hbm,
            xb, x, wqb, wqkv, wob, wo, wrt, wit, wct, wc, wsm, cm, q, hb, ob, T, P, sem):
    cps = [pltpu.make_async_copy(s, d, sem.at[i]) for i, (s, d) in enumerate(
        [(wqkv_hbm.at[:, pl.ds(j * D, D)], wqb.at[:, pl.ds(j * D, D)]) for j in range(3)]
        + [(x_hbm, xb), (wo_hbm, wob), (wr_hbm, wrt), (wi_hbm, wit), (cm_hbm, cm)])]
    cps[0].start()
    cps[3].start()
    for j in range(3):
        cps[j].wait()
        cps[(1, 2, 4)[j]].start()
        _swap_lanes(wqb, wqkv, j * D)
    cps[3].wait()
    cps[4].wait()
    for c in cps[5:]:
        c.start()
    _swap_rows(wob, wo)

    def ldx(rows):
        return jnp.concatenate([x[t, rows, :] for t in range(8)], 1)

    def stx(rows, v):
        for t in range(8):
            x[t, rows, :] = v[:, 128 * t:128 * (t + 1)]

    def cvt(i, _):
        rows = pl.ds(pl.multiple_of(i * 128, 128), 128)
        stx(rows, xb[rows, :].astype(F32))
        return 0
    lax.fori_loop(0, S // 128, cvt, 0)

    def layer_a():
        NC = BS // RC
        CW = 4 * D // NC
        q[0, 8:24, 0:16, :] = jnp.zeros((16, 16, 128), F32)

        def step(i, do_q, do_a, do_o):
            cur = (i + 2) % 2
            nxt = 1 - cur
            if do_q:
                hb[...] = _i32(_ln(ldx(pl.ds(pl.multiple_of((i + 1) * BS, BS), BS))))
                if do_a:
                    q[nxt, 8:24, 0:16, :] = q[cur, 8:24, BS:BS + 16, :]

            def attn(c, mm):
                r0 = pl.multiple_of(c * RC, RC)
                win = pl.ds(r0, RC + 16)
                r2 = []
                acc = [None] * 8
                for t in range(8):
                    ls = slice(128 * t, 128 * (t + 1))
                    if t % 4 == 0:
                        r2.append(mm(t // 4))
                    qq = q[cur, t, pl.ds(r0 + 16, RC), :]
                    for w in range(8):
                        p = qq * q[cur, 8 + t, pl.ds(r0 + 16 - 2 * w, RC), :]
                        acc[w] = p if t == 0 else acc[w] + p
                lg = _dot(jnp.concatenate(acc, 0).astype(BF), _bf(grp[...]))
                pos = i * BS + r0 + lax.broadcasted_iota(jnp.int32, (RC, 128), 0)
                lg = [jnp.where(pos >= 2 * w, lg[w * RC:(w + 1) * RC] * (32 ** -0.5), -1e9) for w in range(8)]
                m = lg[0]
                for w in range(1, 8):
                    m = jnp.maximum(m, lg[w])
                e = [jnp.exp(l - m) for l in lg]
                tot = e[0]
                for w in range(1, 8):
                    tot = tot + e[w]
                inv = 1.0 / tot
                e = [z * inv for z in e]
                for t in range(8):
                    ls = slice(128 * t, 128 * (t + 1))
                    if t % 4 == 0:
                        r2.append(mm(2 + t // 4))
                    o = e[0] * q[cur, 16 + t, pl.ds(r0 + 16, RC), :]
                    for w in range(1, 8):
                        o = o + e[w] * q[cur, 16 + t, pl.ds(r0 + 16 - 2 * w, RC), :]
                    ob[cur, pl.ds(pl.multiple_of(c * (RC // 2), RC // 2), RC // 2), ls] = _i32(o)

                return r2

            HW = CW // 4

            def both(c, ca, do, mm):
                if not do:
                    return attn(ca, lambda j: None)
                return jnp.concatenate(attn(ca, mm) if do_a else [mm(j) for j in range(4)], 1)

            def c1(c, _):
                r = both(c, c, do_q, lambda j: _dot(_bf(hb[...]), _bf(wqkv[:, pl.ds(pl.multiple_of(c * CW + j * HW, HW), HW)])))
                if do_q:
                    for t in range(CW // 128):
                        q[nxt, c * (CW // 128) + t, 16:, :] = r[:, 128 * t:128 * (t + 1)]
                return 0

            def c2(c, _):
                r = both(c, c + 3 * NC // 4, do_o, lambda j: _dot(_bf(ob[nxt]), _bf(wo[:, pl.ds(pl.multiple_of(c * CW + j * HW, HW), HW)])))
                if do_o:
                    rows = pl.ds(pl.multiple_of((i - 1) * BS, BS), BS)
                    for t in range(CW // 128):
                        tt = c * (CW // 128) + t
                        x[tt, rows, :] = x[tt, rows, :] + r[:, 128 * t:128 * (t + 1)]
                return 0
            if do_q or do_a:
                lax.fori_loop(0, 3 * NC // 4, c1, 0)
            if do_o or do_a:
                lax.fori_loop(0, NC // 4, c2, 0)
            return 0
        nb = S // BS
        step(-1, True, False, False)
        step(0, True, True, False)
        lax.fori_loop(1, nb - 1, lambda i, _: step(i, True, True, True), 0)
        step(nb - 1, False, True, True)
        step(nb, False, False, True)

    def layer_b():
        n = GA * 128
        lane = lax.broadcasted_iota(jnp.int32, (128, 128), 1)
        h = float(np.sqrt(0.5))
        P[...] = jnp.zeros((128, 128), F32)

        def fwd(g, _):
            z = _ln(jnp.concatenate(
                [ldx(pl.ds(g * GA + j, 128, stride=16)) for j in range(GA)], 0))
            z = [z[:, 128 * t:128 * (t + 1)] for t in range(8)]
            e = [z[t] + z[t + 4] for t in range(4)]
            o = [z[t] - z[t + 4] for t in range(4)]
            s0, s1 = e[0] + e[2], e[1] + e[3]
            a, b = (o[1] - o[3]) * h, (o[1] + o[3]) * (-h)
            u = [(s0 + s1, s0 - s1), (o[0] + a, b - o[2]),
                 (e[0] - e[2], e[3] - e[1]), (o[0] - a, b + o[2])]
            zz = [_dot(jnp.concatenate(u[p], 1).astype(BF), _bf(cm[p])) for p in range(4)]
            pv = P[...]
            for j in range(GA):
                rs = slice(128 * j, 128 * (j + 1))
                pv = jnp.where(lane == g * GA + j, zz[0][rs, 0:1], pv)
                pv = jnp.where(lane == g * GA + j + 16, zz[0][rs, 128:129], pv)
            P[...] = pv
            zre = jnp.concatenate([v[:, :128] for v in zz], 1).astype(BF)
            zim = jnp.concatenate([v[:, 128:] for v in zz], 1).astype(BF)
            for j in range(GA):
                rs = slice(128 * j, 128 * (j + 1))
                T[g * GA + j] = _dot(_bf(cm[8 + g * GA + j]), jnp.concatenate([zre[rs], zim[rs]], 0))
            return 0
        lax.fori_loop(0, 16 // GA, fwd, 0)

        def wsplit(w):
            return (pltpu.bitcast(w << 16, F32), pltpu.bitcast(w & jnp.int32(-65536), F32))

        g_ = _dot(P[...].T[0:32].astype(BF), _bf(f128[...]))
        gr, gi, tr, ti = g_[:, :128], g_[:, 128:], tw[0:32], tw[32:64]
        g_ = _dot(_bf(f16[0:32]), jnp.concatenate([gr * tr - gi * ti, gr * ti + gi * tr], 0).astype(BF))
        gr, gi = g_[:32], g_[32:]
        ar, ai = wsplit(wsm[...])
        g_ = _dot(_bf(f16[32:64]), jnp.concatenate([gr * ar - gi * ai, gr * ai + gi * ar], 0).astype(BF))
        gr, gi = g_[:32], g_[32:]
        g_ = _dot(jnp.concatenate([gr * tr + gi * ti, gi * tr - gr * ti], 1).astype(BF), _bf(i128[...]))
        P[...] = jnp.concatenate([g_, jnp.zeros((96, 128), F32)], 0).T

        def mid(r, _):
            h0 = pl.multiple_of(r * 8, 8)
            for t in range(4):
                ls = slice(128 * t, 128 * (t + 1))
                v = _fft([(T[a, pl.ds(h0, 8), ls], T[a, pl.ds(h0 + 128, 8), ls]) for a in range(16)], -1)
                y = []
                for k in range(16):
                    a, b = wsplit(wc[pl.ds(h0 + 128 * k, 8), ls])
                    y.append((v[k][0] * a - v[k][1] * b, v[k][0] * b + v[k][1] * a))
                y = _fft(y, 1)
                for a in range(16):
                    T[a, pl.ds(h0, 8), ls] = y[a][0]
                    T[a, pl.ds(h0 + 128, 8), ls] = y[a][1]
            return 0
        lax.fori_loop(0, 16, mid, 0)

        def inv(g, _):
            us = [_dot(_bf(cm[24 + g * GA + j]), T[g * GA + j].astype(BF)) for j in range(GA)]
            pv = P[...]
            G = []
            for p in range(4):
                ls = slice(128 * p, 128 * (p + 1))
                re, im = [v[:128, ls] for v in us], [v[128:, ls] for v in us]
                if p == 0:
                    def col(c):
                        return jnp.sum(jnp.where(lane == c, pv, 0.0), axis=1, keepdims=True)
                    re = [jnp.where(lane == 0, col(g * GA + j), re[j]) for j in range(GA)]
                    im = [jnp.where(lane == 0, col(g * GA + j + 16), im[j]) for j in range(GA)]
                v = _dot(jnp.concatenate([jnp.concatenate(re, 0), jnp.concatenate(im, 0)], 1).astype(BF),
                         _bf(cm[4 + p]))
                G.append((v[:, :128], v[:, 128:]))
            s0, s1 = G[0][0] + G[0][1], G[0][0] - G[0][1]
            e = [s0 + G[2][0], s1 - G[2][1], s0 - G[2][0], s1 + G[2][1]]
            a, b = (G[1][0] - G[3][0]) * h, (G[1][1] + G[3][1]) * (-h)
            o = [G[1][0] + G[3][0], b + a, G[3][1] - G[1][1], b - a]
            for t in range(8):
                y = e[t] + o[t] if t < 4 else e[t - 4] - o[t - 4]
                for j in range(GA):
                    rs = pl.ds(g * GA + j, 128, stride=16)
                    x[t, rs, :] = x[t, rs, :] + y[128 * j:128 * (j + 1)]
            return 0
        lax.fori_loop(0, 16 // GA, inv, 0)

    def pair(p, c):
        layer_a()

        @pl.when(p == 0)
        def _():
            for cp in cps[5:]:
                cp.wait()

            def comb(r, c):
                lo = pltpu.bitcast(wrt[r, c].astype(F32), jnp.int32)
                return lax.shift_right_logical(lo, 16) | pltpu.bitcast(wit[r, c].astype(F32), jnp.int32)

            def tr(j, _):
                rs = pl.ds(pl.multiple_of(j * 128, 128), 128)
                wct[...] = comb(slice(0, 512), rs)
                for t, ks in enumerate(PAIRS):
                    wc[rs, 128 * t:128 * (t + 1)] = jnp.concatenate(
                        [wct[pl.ds(k, 64, stride=8), :] for k in ks], 0).T
                return 0
            lax.fori_loop(0, S // 128, tr, 0)
            for m in range(2):
                row = comb(slice(512 * m, 512 * m + 1), slice(None))
                for k in range(16):
                    wsm[16 * m + k:16 * m + k + 1, :] = row[:, 128 * k:128 * (k + 1)]
        layer_b()
        return c
    lax.fori_loop(0, 2, pair, 0)

    outs = []
    for i in range(4):
        rows = pl.ds(i * 512, 512)
        xb[rows, :] = ldx(rows).astype(BF)
        c = pltpu.make_async_copy(xb.at[rows], out_hbm.at[rows], sem.at[i])
        c.start()
        outs.append(c)
    for c in outs:
        c.wait()


@jax.jit
def pallas_interleave_layers__sliding_local_dilated__spectral_gfnet__prompt_kernel(
    A_x, A_wqkv, A_wo, B_x, B_w_r, B_w_i):
    consts = _consts()
    I32 = jnp.int32
    anyspec = pl.BlockSpec(memory_space=pl.ANY)
    V = pltpu.VMEM
    out = pl.pallas_call(
        _kernel,
        out_shape=jax.ShapeDtypeStruct((S, D), BF),
        in_specs=[anyspec] * 6 + [pl.BlockSpec(memory_space=V)] * 5,
        out_specs=anyspec,
        scratch_shapes=[
            V((S, D), BF), V((8, S, 128), F32),
            V((D, 3 * D), BF), V((D // 2, 3 * D), I32), V((D, D), BF), V((D // 2, D), I32),
            V((513, S), BF), V((513, S), BF), V((512, 128), I32), V((S, 512), I32), V((32, 128), I32),
            V(consts[0].shape, I32),
            V((2, 24, BS + 16, 128), F32), V((BS // 2, D), I32), V((2, BS // 2, D), I32),
            V((16, 256, 512), F32), V((128, 128), F32), pltpu.SemaphoreType.DMA((8,))],
        compiler_params=pltpu.CompilerParams(vmem_limit_bytes=110 * 2 ** 20),
    )(A_x.reshape(S, D), A_wqkv, A_wo, B_w_r.T, B_w_i.T, *consts)
    return out.reshape(1, S, D)
```

```python
import numpy as np
import jax
import jax.numpy as jnp
from jax import lax
import jax.experimental.pallas as pl
import jax.experimental.pallas.tpu as pltpu

S, D = 2048, 1024
BS = 256
RC = 64
GA = 4
F32, BF = jnp.float32, jnp.bfloat16


PAIRS = ((0, 4), (1, 7), (2, 6), (3, 5))


def _pack(m):
    u = m.astype(np.float32).astype(BF).view(np.uint16).astype(np.uint32)
    return (u[..., 0::2, :] | (u[..., 1::2, :] << 16)).view(np.int32)


def _consts():
    l = np.arange(128)
    b, j = l[:, None], np.arange(64)[None, :]
    df = np.zeros((4, 256, 256)); di = np.zeros((4, 256, 256))
    for p, (ka, kb) in enumerate(PAIRS):
        ta, tb = (2 * np.pi * b * (k + 8 * j) / 1024 for k in (ka, kb))
        ca, sa, cb, sb = np.cos(ta), np.sin(ta), np.cos(tb), np.sin(tb)
        if p == 0:
            sa[:, 0] = -(-1.0) ** l
            df[p] = np.block([[ca, 0 * ca, -sa, 0 * ca], [0 * ca, cb, 0 * ca, -sb]])
        else:
            df[p] = np.block([[ca, cb, -sa, -sb], [sa, -sb, ca, -cb]])
        di[p] = 2 * df[p].T
    di[0, [0, 128]] /= 2
    grp = (l[:, None] // 4 == l[None, :] // 4) * 1.0
    mf = np.zeros((16, 256, 256)); mi = np.zeros((16, 256, 256))
    for a in range(16):
        t = 2 * np.pi * l[:, None] * (a + 16 * l[None, :]) / 2048
        c, s = np.cos(t), np.sin(t)
        mf[a] = np.block([[c, s], [-s, c]])
        mi[a] = np.block([[c.T, -s.T], [s.T, c.T]]) / (S * D)
    t = 2 * np.pi * l[:, None] * l[None, :] / 128
    f128 = np.concatenate([np.cos(t), -np.sin(t)], 1)
    i128 = f128.T / (S * D)
    r = np.arange(32)
    t = 2 * np.pi * (r[:, None] % 16) * l[None, :] / 2048
    tw = np.concatenate([np.cos(t), -np.sin(t)], 0).astype(np.float32)
    t = 2 * np.pi * (r[:, None] % 16) * (r[None, :] % 16) / 16
    same = r[:, None] // 16 == r[None, :] // 16
    c, s = np.cos(t) * same, np.sin(t) * same
    f16 = np.block([[c, s], [-s, c]])
    return (_pack(np.concatenate([df, di, mf, mi], 0)), _pack(grp), _pack(f128), _pack(i128),
            _pack(np.concatenate([f16, f16.T], 0)), tw)


def _bf(v):
    return pltpu.bitcast(v, BF)


def _i32(v):
    return pltpu.bitcast(v.astype(BF), jnp.int32)


def _dot(a, b):
    return jnp.dot(a, b, preferred_element_type=F32)


def _ln(x):
    m = jnp.mean(x, axis=-1, keepdims=True)
    xc = x - m
    v = jnp.mean(xc * xc, axis=-1, keepdims=True)
    return xc * lax.rsqrt(v + 1e-5)


def _fft(v, sign):
    n = len(v)
    if n == 1:
        return v
    e, o = _fft(v[0::2], sign), _fft(v[1::2], sign)
    out = [None] * n
    for k in range(n // 2):
        er, ei = e[k]
        r, i = o[k]
        if k == 0:
            out[k], out[k + n // 2] = (er + r, ei + i), (er - r, ei - i)
        elif 4 * k == n:
            if sign > 0:
                out[k], out[k + n // 2] = (er - i, ei + r), (er + i, ei - r)
            else:
                out[k], out[k + n // 2] = (er + i, ei - r), (er - i, ei + r)
        else:
            c = float(np.cos(2 * np.pi * k / n)); s = float(sign * np.sin(2 * np.pi * k / n))
            if 8 * k == n or 8 * k == 3 * n:
                h = abs(c)
                if c > 0 and s > 0: tr, ti = (r - i) * h, (r + i) * h
                elif c > 0: tr, ti = (r + i) * h, (i - r) * h
                elif s > 0: tr, ti = (r + i) * (-h), (r - i) * h
                else: tr, ti = (i - r) * h, (r + i) * (-h)
            else:
                tr, ti = r * c - i * s, r * s + i * c
            out[k], out[k + n // 2] = (er + tr, ei + ti), (er - tr, ei - ti)
    return out


def _swap_lanes(w_ref, o_ref, c0):
    def body(r, _):
        rows = pl.ds(pl.multiple_of(r * 64, 64), 64)
        t = [pltpu.bitcast(w_ref[rows, c0 + 128 * u:c0 + 128 * (u + 1)], jnp.int32) for u in range(8)]
        lane = lax.broadcasted_iota(jnp.int32, (32, 128), 1)
        for bit in range(3):
            dist = 4 << bit
            lo = (lane & dist) == 0
            for u in range(8):
                if not u & (1 << bit):
                    a, b = t[u], t[u | (1 << bit)]
                    t[u] = jnp.where(lo, a, pltpu.roll(b, dist, 1))
                    t[u | (1 << bit)] = jnp.where(lo, pltpu.roll(a, 128 - dist, 1), b)
        for u in range(8):
            o_ref[pl.ds(pl.multiple_of(r * 32, 32), 32), c0 + 128 * u:c0 + 128 * (u + 1)] = t[u]
        return 0
    lax.fori_loop(0, D // 64, body, 0)


def _swap_rows(w_ref, o_ref):
    def body(c, _):
        cols = pl.ds(pl.multiple_of(c * 128, 128), 128)
        t = [pltpu.bitcast(w_ref[128 * u:128 * (u + 1), cols], jnp.int32) for u in range(8)]
        row = lax.broadcasted_iota(jnp.int32, (64, 128), 0)
        for bit in range(3):
            dist = 2 << bit
            lo = (row & dist) == 0
            for u in range(8):
                if not u & (1 << bit):
                    a, b = t[u], t[u | (1 << bit)]
                    t[u] = jnp.where(lo, a, pltpu.roll(b, dist, 0))
                    t[u | (1 << bit)] = jnp.where(lo, pltpu.roll(a, 64 - dist, 0), b)
        for u in range(8):
            o_ref[64 * u:64 * (u + 1), cols] = t[u]
        return 0
    lax.fori_loop(0, D // 128, body, 0)


def _kernel(x_hbm, wqkv_hbm, wo_hbm, wr_hbm, wi_hbm, cm_hbm, grp, f128, i128, f16, tw, out_hbm,
            xb, x, wqb, wqkv, wob, wo, wrt, wit, wct, wc, wsm, cm, q, hb, ob, T, P, sem):
    cps = [pltpu.make_async_copy(s, d, sem.at[i]) for i, (s, d) in enumerate(
        [(wqkv_hbm.at[:, pl.ds(j * D, D)], wqb.at[:, pl.ds(j * D, D)]) for j in range(3)]
        + [(x_hbm, xb), (wo_hbm, wob), (wr_hbm, wrt), (wi_hbm, wit), (cm_hbm, cm)])]
    cps[0].start()
    cps[3].start()
    for j in range(3):
        cps[j].wait()
        cps[(1, 2, 4)[j]].start()
        _swap_lanes(wqb, wqkv, j * D)
    cps[3].wait()
    cps[4].wait()
    for c in cps[5:]:
        c.start()
    _swap_rows(wob, wo)

    def ldx(rows):
        return jnp.concatenate([x[t, rows, :] for t in range(8)], 1)

    def grp16(m):
        return pl.ds(m * 17, 16)

    def ldb(m0, n):
        return jnp.concatenate([ldx(grp16(m0 + m)) for m in range(n // 16)], 0)

    def stx(rows, v):
        for t in range(8):
            x[t, rows, :] = v[:, 128 * t:128 * (t + 1)]

    def cvt(i, _):
        for m in range(8):
            stx(grp16(i * 8 + m), xb[pl.ds(pl.multiple_of(i * 128 + m * 16, 16), 16), :].astype(F32))
        return 0
    lax.fori_loop(0, S // 128, cvt, 0)

    def layer_a():
        NC = BS // RC
        CW = 4 * D // NC
        q[0, 8:24, 0:16, :] = jnp.zeros((16, 16, 128), F32)

        def step(i, do_q, do_a, do_o):
            cur = (i + 2) % 2
            nxt = 1 - cur
            if do_q:
                hb[...] = _i32(_ln(ldb((i + 1) * (BS // 16), BS)))
                if do_a:
                    q[nxt, 8:24, 0:16, :] = q[cur, 8:24, BS:BS + 16, :]

            def attn(c, mm):
                r0 = pl.multiple_of(c * RC, RC)
                win = pl.ds(r0, RC + 16)
                r2 = []
                acc = [None] * 8
                for t in range(8):
                    ls = slice(128 * t, 128 * (t + 1))
                    if t % 4 == 0:
                        r2.append(mm(t // 4))
                    qq = q[cur, t, pl.ds(r0 + 16, RC), :]
                    for w in range(8):
                        p = qq * q[cur, 8 + t, pl.ds(r0 + 16 - 2 * w, RC), :]
                        acc[w] = p if t == 0 else acc[w] + p
                lg = _dot(jnp.concatenate(acc, 0).astype(BF), _bf(grp[...]))
                pos = i * BS + r0 + lax.broadcasted_iota(jnp.int32, (RC, 128), 0)
                lg = [jnp.where(pos >= 2 * w, lg[w * RC:(w + 1) * RC] * (32 ** -0.5), -1e9) for w in range(8)]
                m = lg[0]
                for w in range(1, 8):
                    m = jnp.maximum(m, lg[w])
                e = [jnp.exp(l - m) for l in lg]
                tot = e[0]
                for w in range(1, 8):
                    tot = tot + e[w]
                inv = 1.0 / tot
                e = [z * inv for z in e]
                for t in range(8):
                    ls = slice(128 * t, 128 * (t + 1))
                    if t % 4 == 0:
                        r2.append(mm(2 + t // 4))
                    o = e[0] * q[cur, 16 + t, pl.ds(r0 + 16, RC), :]
                    for w in range(1, 8):
                        o = o + e[w] * q[cur, 16 + t, pl.ds(r0 + 16 - 2 * w, RC), :]
                    ob[cur, pl.ds(pl.multiple_of(c * (RC // 2), RC // 2), RC // 2), ls] = _i32(o)

                return r2

            HW = CW // 4

            def both(ca, do, mm):
                if do_a:
                    attn(ca, mm if do else lambda j: None)
                else:
                    for j in range(4):
                        mm(j)
                return 0

            def c1(c, _):
                def mm(j):
                    r = _dot(_bf(hb[...]), _bf(wqkv[:, pl.ds(pl.multiple_of(c * CW + j * HW, HW), HW)]))
                    for t in range(HW // 128):
                        q[nxt, (c * CW + j * HW) // 128 + t, 16:, :] = r[:, 128 * t:128 * (t + 1)]
                return both(c, do_q, mm)

            def c2(c, _):
                def mm(j):
                    r = _dot(_bf(ob[nxt]), _bf(wo[:, pl.ds(pl.multiple_of(c * CW + j * HW, HW), HW)]))
                    for t in range(HW // 128):
                        tt = (c * CW + j * HW) // 128 + t
                        for m in range(BS // 16):
                            rows = grp16((i - 1) * (BS // 16) + m)
                            x[tt, rows, :] = x[tt, rows, :] + r[16 * m:16 * m + 16, 128 * t:128 * (t + 1)]
                return both(c + 3 * NC // 4, do_o, mm)
            if do_q or do_a:
                lax.fori_loop(0, 3 * NC // 4, c1, 0)
            if do_o or do_a:
                lax.fori_loop(0, NC // 4, c2, 0)
            return 0
        nb = S // BS
        step(-1, True, False, False)
        step(0, True, True, False)
        lax.fori_loop(1, nb - 1, lambda i, _: step(i, True, True, True), 0)
        step(nb - 1, False, True, True)
        step(nb, False, False, True)

    def layer_b():
        n = GA * 128
        lane = lax.broadcasted_iota(jnp.int32, (128, 128), 1)
        h = float(np.sqrt(0.5))
        P[...] = jnp.zeros((128, 128), F32)

        def fwd(g, _):
            z = _ln(jnp.concatenate(
                [ldx(pl.ds(g * GA + j, 128, stride=17)) for j in range(GA)], 0))
            z = [z[:, 128 * t:128 * (t + 1)] for t in range(8)]
            e = [z[t] + z[t + 4] for t in range(4)]
            o = [z[t] - z[t + 4] for t in range(4)]
            s0, s1 = e[0] + e[2], e[1] + e[3]
            a, b = (o[1] - o[3]) * h, (o[1] + o[3]) * (-h)
            u = [(s0 + s1, s0 - s1), (o[0] + a, b - o[2]),
                 (e[0] - e[2], e[3] - e[1]), (o[0] - a, b + o[2])]
            zz = [_dot(jnp.concatenate(u[p], 1).astype(BF), _bf(cm[p])) for p in range(4)]
            pv = P[...]
            for j in range(GA):
                rs = slice(128 * j, 128 * (j + 1))
                pv = jnp.where(lane == g * GA + j, zz[0][rs, 0:1], pv)
                pv = jnp.where(lane == g * GA + j + 16, zz[0][rs, 128:129], pv)
            P[...] = pv
            zre = jnp.concatenate([v[:, :128] for v in zz], 1).astype(BF)
            zim = jnp.concatenate([v[:, 128:] for v in zz], 1).astype(BF)
            for j in range(GA):
                rs = slice(128 * j, 128 * (j + 1))
                T[g * GA + j] = _dot(_bf(cm[8 + g * GA + j]), jnp.concatenate([zre[rs], zim[rs]], 0))
            return 0
        lax.fori_loop(0, 16 // GA, fwd, 0)

        def wsplit(w):
            return (pltpu.bitcast(w << 16, F32), pltpu.bitcast(w & jnp.int32(-65536), F32))

        g_ = _dot(P[...].T[0:32].astype(BF), _bf(f128[...]))
        gr, gi, tr, ti = g_[:, :128], g_[:, 128:], tw[0:32], tw[32:64]
        g_ = _dot(_bf(f16[0:32]), jnp.concatenate([gr * tr - gi * ti, gr * ti + gi * tr], 0).astype(BF))
        gr, gi = g_[:32], g_[32:]
        ar, ai = wsplit(wsm[...])
        g_ = _dot(_bf(f16[32:64]), jnp.concatenate([gr * ar - gi * ai, gr * ai + gi * ar], 0).astype(BF))
        gr, gi = g_[:32], g_[32:]
        g_ = _dot(jnp.concatenate([gr * tr + gi * ti, gi * tr - gr * ti], 1).astype(BF), _bf(i128[...]))
        P[...] = jnp.concatenate([g_, jnp.zeros((96, 128), F32)], 0).T

        def mid(r, _):
            h0 = pl.multiple_of(r * 8, 8)
            for t in range(4):
                ls = slice(128 * t, 128 * (t + 1))
                v = _fft([(T[a, pl.ds(h0, 8), ls], T[a, pl.ds(h0 + 128, 8), ls]) for a in range(16)], -1)
                y = []
                for k in range(16):
                    a, b = wsplit(wc[pl.ds(h0 + 128 * k, 8), ls])
                    y.append((v[k][0] * a - v[k][1] * b, v[k][0] * b + v[k][1] * a))
                y = _fft(y, 1)
                for a in range(16):
                    T[a, pl.ds(h0, 8), ls] = y[a][0]
                    T[a, pl.ds(h0 + 128, 8), ls] = y[a][1]
            return 0
        lax.fori_loop(0, 16, mid, 0)

        def inv(g, _):
            us = [_dot(_bf(cm[24 + g * GA + j]), T[g * GA + j].astype(BF)) for j in range(GA)]
            pv = P[...]
            G = []
            for p in range(4):
                ls = slice(128 * p, 128 * (p + 1))
                re, im = [v[:128, ls] for v in us], [v[128:, ls] for v in us]
                if p == 0:
                    def col(c):
                        return jnp.sum(jnp.where(lane == c, pv, 0.0), axis=1, keepdims=True)
                    re = [jnp.where(lane == 0, col(g * GA + j), re[j]) for j in range(GA)]
                    im = [jnp.where(lane == 0, col(g * GA + j + 16), im[j]) for j in range(GA)]
                v = _dot(jnp.concatenate([jnp.concatenate(re, 0), jnp.concatenate(im, 0)], 1).astype(BF),
                         _bf(cm[4 + p]))
                G.append((v[:, :128], v[:, 128:]))
            s0, s1 = G[0][0] + G[0][1], G[0][0] - G[0][1]
            e = [s0 + G[2][0], s1 - G[2][1], s0 - G[2][0], s1 + G[2][1]]
            a, b = (G[1][0] - G[3][0]) * h, (G[1][1] + G[3][1]) * (-h)
            o = [G[1][0] + G[3][0], b + a, G[3][1] - G[1][1], b - a]
            for t in range(8):
                y = e[t] + o[t] if t < 4 else e[t - 4] - o[t - 4]
                for j in range(GA):
                    rs = pl.ds(g * GA + j, 128, stride=17)
                    x[t, rs, :] = x[t, rs, :] + y[128 * j:128 * (j + 1)]
            return 0
        lax.fori_loop(0, 16 // GA, inv, 0)

    def pair(p, c):
        layer_a()

        @pl.when(p == 0)
        def _():
            for cp in cps[5:]:
                cp.wait()

            def comb(r, c):
                lo = pltpu.bitcast(wrt[r, c].astype(F32), jnp.int32)
                return lax.shift_right_logical(lo, 16) | pltpu.bitcast(wit[r, c].astype(F32), jnp.int32)

            def tr(j, _):
                rs = pl.ds(pl.multiple_of(j * 128, 128), 128)
                wct[...] = comb(slice(0, 512), rs)
                for t, ks in enumerate(PAIRS):
                    wc[rs, 128 * t:128 * (t + 1)] = jnp.concatenate(
                        [wct[pl.ds(k, 64, stride=8), :] for k in ks], 0).T
                return 0
            lax.fori_loop(0, S // 128, tr, 0)
            for m in range(2):
                row = comb(slice(512 * m, 512 * m + 1), slice(None))
                for k in range(16):
                    wsm[16 * m + k:16 * m + k + 1, :] = row[:, 128 * k:128 * (k + 1)]
        layer_b()
        return c
    lax.fori_loop(0, 2, pair, 0)

    outs = []
    for i in range(4):
        rows = pl.ds(i * 512, 512)
        xb[rows, :] = ldb(i * 32, 512).astype(BF)
        c = pltpu.make_async_copy(xb.at[rows], out_hbm.at[rows], sem.at[i])
        c.start()
        outs.append(c)
    for c in outs:
        c.wait()


@jax.jit
def pallas_interleave_layers__sliding_local_dilated__spectral_gfnet__prompt_kernel(
    A_x, A_wqkv, A_wo, B_x, B_w_r, B_w_i):
    consts = _consts()
    I32 = jnp.int32
    anyspec = pl.BlockSpec(memory_space=pl.ANY)
    V = pltpu.VMEM
    out = pl.pallas_call(
        _kernel,
        out_shape=jax.ShapeDtypeStruct((S, D), BF),
        in_specs=[anyspec] * 6 + [pl.BlockSpec(memory_space=V)] * 5,
        out_specs=anyspec,
        scratch_shapes=[
            V((S, D), BF), V((8, S // 16 * 17, 128), F32),
            V((D, 3 * D), BF), V((D // 2, 3 * D), I32), V((D, D), BF), V((D // 2, D), I32),
            V((513, S), BF), V((513, S), BF), V((512, 128), I32), V((S, 512), I32), V((32, 128), I32),
            V(consts[0].shape, I32),
            V((2, 24, BS + 16, 128), F32), V((BS // 2, D), I32), V((2, BS // 2, D), I32),
            V((16, 256, 512), F32), V((128, 128), F32), pltpu.SemaphoreType.DMA((8,))],
        compiler_params=pltpu.CompilerParams(vmem_limit_bytes=110 * 2 ** 20),
    )(A_x.reshape(S, D), A_wqkv, A_wo, B_w_r.T, B_w_i.T, *consts)
    return out.reshape(1, S, D)
```

```python
import numpy as np
import jax
import jax.numpy as jnp
from jax import lax
import jax.experimental.pallas as pl
import jax.experimental.pallas.tpu as pltpu

S, D = 2048, 1024
BS = 512
RC = 128
GA = 4
F32, BF = jnp.float32, jnp.bfloat16


PAIRS = ((0, 4), (1, 7), (2, 6), (3, 5))


def _pack(m):
    u = m.astype(np.float32).astype(BF).view(np.uint16).astype(np.uint32)
    return (u[..., 0::2, :] | (u[..., 1::2, :] << 16)).view(np.int32)


def _consts():
    l = np.arange(128)
    b, j = l[:, None], np.arange(64)[None, :]
    df = np.zeros((4, 256, 256)); di = np.zeros((4, 256, 256))
    for p, (ka, kb) in enumerate(PAIRS):
        ta, tb = (2 * np.pi * b * (k + 8 * j) / 1024 for k in (ka, kb))
        ca, sa, cb, sb = np.cos(ta), np.sin(ta), np.cos(tb), np.sin(tb)
        if p == 0:
            sa[:, 0] = -(-1.0) ** l
            df[p] = np.block([[ca, 0 * ca, -sa, 0 * ca], [0 * ca, cb, 0 * ca, -sb]])
        else:
            df[p] = np.block([[ca, cb, -sa, -sb], [sa, -sb, ca, -cb]])
        di[p] = 2 * df[p].T
    di[0, [0, 128]] /= 2
    grp = (l[:, None] // 4 == l[None, :] // 4) * 1.0
    mf = np.zeros((16, 256, 256)); mi = np.zeros((16, 256, 256))
    for a in range(16):
        t = 2 * np.pi * l[:, None] * (a + 16 * l[None, :]) / 2048
        c, s = np.cos(t), np.sin(t)
        mf[a] = np.block([[c, s], [-s, c]])
        mi[a] = np.block([[c.T, -s.T], [s.T, c.T]]) / (S * D)
    t = 2 * np.pi * l[:, None] * l[None, :] / 128
    f128 = np.concatenate([np.cos(t), -np.sin(t)], 1)
    i128 = f128.T / (S * D)
    r = np.arange(32)
    t = 2 * np.pi * (r[:, None] % 16) * l[None, :] / 2048
    tw = np.concatenate([np.cos(t), -np.sin(t)], 0).astype(np.float32)
    t = 2 * np.pi * (r[:, None] % 16) * (r[None, :] % 16) / 16
    same = r[:, None] // 16 == r[None, :] // 16
    c, s = np.cos(t) * same, np.sin(t) * same
    f16 = np.block([[c, s], [-s, c]])
    return (_pack(np.concatenate([df, di, mf, mi], 0)), _pack(grp), _pack(f128), _pack(i128),
            _pack(np.concatenate([f16, f16.T], 0)), tw)


def _bf(v):
    return pltpu.bitcast(v, BF)


def _i32(v):
    return pltpu.bitcast(v.astype(BF), jnp.int32)


def _dot(a, b):
    return jnp.dot(a, b, preferred_element_type=F32)


def _ln(x):
    m = jnp.mean(x, axis=-1, keepdims=True)
    xc = x - m
    v = jnp.mean(xc * xc, axis=-1, keepdims=True)
    return xc * lax.rsqrt(v + 1e-5)


def _fft(v, sign):
    n = len(v)
    if n == 1:
        return v
    e, o = _fft(v[0::2], sign), _fft(v[1::2], sign)
    out = [None] * n
    for k in range(n // 2):
        er, ei = e[k]
        r, i = o[k]
        if k == 0:
            out[k], out[k + n // 2] = (er + r, ei + i), (er - r, ei - i)
        elif 4 * k == n:
            if sign > 0:
                out[k], out[k + n // 2] = (er - i, ei + r), (er + i, ei - r)
            else:
                out[k], out[k + n // 2] = (er + i, ei - r), (er - i, ei + r)
        else:
            c = float(np.cos(2 * np.pi * k / n)); s = float(sign * np.sin(2 * np.pi * k / n))
            if 8 * k == n or 8 * k == 3 * n:
                h = abs(c)
                if c > 0 and s > 0: tr, ti = (r - i) * h, (r + i) * h
                elif c > 0: tr, ti = (r + i) * h, (i - r) * h
                elif s > 0: tr, ti = (r + i) * (-h), (r - i) * h
                else: tr, ti = (i - r) * h, (r + i) * (-h)
            else:
                tr, ti = r * c - i * s, r * s + i * c
            out[k], out[k + n // 2] = (er + tr, ei + ti), (er - tr, ei - ti)
    return out


def _swap_lanes(w_ref, o_ref, c0):
    def body(r, _):
        rows = pl.ds(pl.multiple_of(r * 128, 128), 128)
        t = [pltpu.bitcast(w_ref[rows, c0 + 128 * u:c0 + 128 * (u + 1)], jnp.int32) for u in range(8)]
        lane = lax.broadcasted_iota(jnp.int32, (64, 128), 1)
        for bit in range(3):
            dist = 4 << bit
            lo = (lane & dist) == 0
            for u in range(8):
                if not u & (1 << bit):
                    a, b = t[u], t[u | (1 << bit)]
                    t[u] = jnp.where(lo, a, pltpu.roll(b, dist, 1))
                    t[u | (1 << bit)] = jnp.where(lo, pltpu.roll(a, 128 - dist, 1), b)
        for u in range(8):
            o_ref[pl.ds(pl.multiple_of(r * 64, 64), 64), c0 + 128 * u:c0 + 128 * (u + 1)] = t[u]
        return 0
    lax.fori_loop(0, D // 128, body, 0)


def _swap_rows(w_ref, o_ref):
    def body(c, _):
        cols = pl.ds(pl.multiple_of(c * 128, 128), 128)
        t = [pltpu.bitcast(w_ref[128 * u:128 * (u + 1), cols], jnp.int32) for u in range(8)]
        row = lax.broadcasted_iota(jnp.int32, (64, 128), 0)
        for bit in range(3):
            dist = 2 << bit
            lo = (row & dist) == 0
            for u in range(8):
                if not u & (1 << bit):
                    a, b = t[u], t[u | (1 << bit)]
                    t[u] = jnp.where(lo, a, pltpu.roll(b, dist, 0))
                    t[u | (1 << bit)] = jnp.where(lo, pltpu.roll(a, 64 - dist, 0), b)
        for u in range(8):
            o_ref[64 * u:64 * (u + 1), cols] = t[u]
        return 0
    lax.fori_loop(0, D // 128, body, 0)


def _kernel(x_hbm, wqkv_hbm, wo_hbm, wr_hbm, wi_hbm, cm_hbm, grp, f128, i128, f16, tw, out_hbm,
            xb, x, wqb, wqkv, wob, wo, wrt, wit, wct, wc, wsm, cm, q, hb, ob, T, P, sem):
    cps = [pltpu.make_async_copy(s, d, sem.at[i]) for i, (s, d) in enumerate(
        [(wqkv_hbm.at[:, pl.ds(j * D, D)], wqb.at[:, pl.ds(j * D, D)]) for j in range(3)]
        + [(x_hbm, xb), (wo_hbm, wob), (wr_hbm, wrt), (wi_hbm, wit), (cm_hbm, cm)])]
    cps[3].start()
    cps[0].start()

    def ldx(rows):
        return jnp.concatenate([x[t, rows, :] for t in range(8)], 1)

    def grp16(m):
        return pl.ds(m * 17, 16)

    def ldb(m0, n):
        return jnp.concatenate([ldx(grp16(m0 + m)) for m in range(n // 16)], 0)

    def stx(rows, v):
        for t in range(8):
            x[t, rows, :] = v[:, 128 * t:128 * (t + 1)]

    def cvt(i, _):
        for m in range(8):
            stx(grp16(i * 8 + m), xb[pl.ds(pl.multiple_of(i * 128 + m * 16, 16), 16), :].astype(F32))
        return 0
    cps[3].wait()
    lax.fori_loop(0, S // 128, cvt, 0)
    for j in range(3):
        cps[j].wait()
        cps[(1, 2, 4)[j]].start()
        _swap_lanes(wqb, wqkv, j * D)
    cps[4].wait()
    for c in cps[5:]:
        c.start()
    _swap_rows(wob, wo)


    def layer_a():
        NC = BS // RC
        CW = 4 * D // NC
        q[0, 8:24, 0:16, :] = jnp.zeros((16, 16, 128), F32)

        def step(i, do_q, do_a, do_o):
            cur = (i + 2) % 2
            nxt = 1 - cur
            if do_q:
                hb[...] = _i32(_ln(ldb((i + 1) * (BS // 16), BS)))
                if do_a:
                    q[nxt, 8:24, 0:16, :] = q[cur, 8:24, BS:BS + 16, :]

            def attn(c, mm):
                r0 = pl.multiple_of(c * RC, RC)
                win = pl.ds(r0, RC + 16)
                r2 = []
                acc = [None] * 8
                for t in range(8):
                    ls = slice(128 * t, 128 * (t + 1))
                    if t % 4 == 0:
                        r2.append(mm(t // 4))
                    qq = q[cur, t, pl.ds(r0 + 16, RC), :]
                    for w in range(8):
                        p = qq * q[cur, 8 + t, pl.ds(r0 + 16 - 2 * w, RC), :]
                        acc[w] = p if t == 0 else acc[w] + p
                lg = _dot(jnp.concatenate(acc, 0).astype(BF), _bf(grp[...]))
                pos = i * BS + r0 + lax.broadcasted_iota(jnp.int32, (RC, 128), 0)
                lg = [jnp.where(pos >= 2 * w, lg[w * RC:(w + 1) * RC] * (32 ** -0.5), -1e9) for w in range(8)]
                m = lg[0]
                for w in range(1, 8):
                    m = jnp.maximum(m, lg[w])
                e = [jnp.exp(l - m) for l in lg]
                tot = e[0]
                for w in range(1, 8):
                    tot = tot + e[w]
                inv = 1.0 / tot
                e = [z * inv for z in e]
                for t in range(8):
                    ls = slice(128 * t, 128 * (t + 1))
                    if t % 4 == 0:
                        r2.append(mm(2 + t // 4))
                    o = e[0] * q[cur, 16 + t, pl.ds(r0 + 16, RC), :]
                    for w in range(1, 8):
                        o = o + e[w] * q[cur, 16 + t, pl.ds(r0 + 16 - 2 * w, RC), :]
                    ob[cur, pl.ds(pl.multiple_of(c * (RC // 2), RC // 2), RC // 2), ls] = _i32(o)

                return r2

            HW = CW // 4

            def both(ca, do, mm):
                if do_a:
                    attn(ca, mm if do else lambda j: None)
                else:
                    for j in range(4):
                        mm(j)
                return 0

            def c1(c, _):
                def mm(j):
                    r = _dot(_bf(hb[...]), _bf(wqkv[:, pl.ds(pl.multiple_of(c * CW + j * HW, HW), HW)]))
                    for t in range(HW // 128):
                        q[nxt, (c * CW + j * HW) // 128 + t, 16:, :] = r[:, 128 * t:128 * (t + 1)]
                return both(c, do_q, mm)

            def c2(c, _):
                def mm(j):
                    r = _dot(_bf(ob[nxt]), _bf(wo[:, pl.ds(pl.multiple_of(c * CW + j * HW, HW), HW)]))
                    for t in range(HW // 128):
                        tt = (c * CW + j * HW) // 128 + t
                        for m in range(BS // 16):
                            rows = grp16((i - 1) * (BS // 16) + m)
                            x[tt, rows, :] = x[tt, rows, :] + r[16 * m:16 * m + 16, 128 * t:128 * (t + 1)]
                return both(c + 3 * NC // 4, do_o, mm)
            if do_q or do_a:
                lax.fori_loop(0, 3 * NC // 4, c1, 0)
            if do_o or do_a:
                lax.fori_loop(0, NC // 4, c2, 0)
            return 0
        nb = S // BS
        step(-1, True, False, False)
        step(0, True, True, False)
        lax.fori_loop(1, nb - 1, lambda i, _: step(i, True, True, True), 0)
        step(nb - 1, False, True, True)
        step(nb, False, False, True)

    def layer_b():
        n = GA * 128
        lane = lax.broadcasted_iota(jnp.int32, (128, 128), 1)
        h = float(np.sqrt(0.5))
        P[...] = jnp.zeros((128, 128), F32)

        def fwd(g, _):
            z = _ln(jnp.concatenate(
                [ldx(pl.ds(g * GA + j, 128, stride=17)) for j in range(GA)], 0))
            z = [z[:, 128 * t:128 * (t + 1)] for t in range(8)]
            e = [z[t] + z[t + 4] for t in range(4)]
            o = [z[t] - z[t + 4] for t in range(4)]
            s0, s1 = e[0] + e[2], e[1] + e[3]
            a, b = (o[1] - o[3]) * h, (o[1] + o[3]) * (-h)
            u = [(s0 + s1, s0 - s1), (o[0] + a, b - o[2]),
                 (e[0] - e[2], e[3] - e[1]), (o[0] - a, b + o[2])]
            zz = [_dot(jnp.concatenate(u[p], 1).astype(BF), _bf(cm[p])) for p in range(4)]
            pv = P[...]
            for j in range(GA):
                rs = slice(128 * j, 128 * (j + 1))
                pv = jnp.where(lane == g * GA + j, zz[0][rs, 0:1], pv)
                pv = jnp.where(lane == g * GA + j + 16, zz[0][rs, 128:129], pv)
            P[...] = pv
            zre = jnp.concatenate([v[:, :128] for v in zz], 1).astype(BF)
            zim = jnp.concatenate([v[:, 128:] for v in zz], 1).astype(BF)
            for j in range(GA):
                rs = slice(128 * j, 128 * (j + 1))
                T[g * GA + j] = _dot(_bf(cm[8 + g * GA + j]), jnp.concatenate([zre[rs], zim[rs]], 0))
            return 0
        lax.fori_loop(0, 16 // GA, fwd, 0)

        def wsplit(w):
            return (pltpu.bitcast(w << 16, F32), pltpu.bitcast(w & jnp.int32(-65536), F32))

        g_ = _dot(P[...].T[0:32].astype(BF), _bf(f128[...]))
        gr, gi, tr, ti = g_[:, :128], g_[:, 128:], tw[0:32], tw[32:64]
        g_ = _dot(_bf(f16[0:32]), jnp.concatenate([gr * tr - gi * ti, gr * ti + gi * tr], 0).astype(BF))
        gr, gi = g_[:32], g_[32:]
        ar, ai = wsplit(wsm[...])
        g_ = _dot(_bf(f16[32:64]), jnp.concatenate([gr * ar - gi * ai, gr * ai + gi * ar], 0).astype(BF))
        gr, gi = g_[:32], g_[32:]
        g_ = _dot(jnp.concatenate([gr * tr + gi * ti, gi * tr - gr * ti], 1).astype(BF), _bf(i128[...]))
        P[...] = jnp.concatenate([g_, jnp.zeros((96, 128), F32)], 0).T

        def mid(r, _):
            h0 = pl.multiple_of(r * 8, 8)
            for t in range(4):
                ls = slice(128 * t, 128 * (t + 1))
                v = _fft([(T[a, pl.ds(h0, 8), ls], T[a, pl.ds(h0 + 128, 8), ls]) for a in range(16)], -1)
                y = []
                for k in range(16):
                    a, b = wsplit(wc[pl.ds(h0 + 128 * k, 8), ls])
                    y.append((v[k][0] * a - v[k][1] * b, v[k][0] * b + v[k][1] * a))
                y = _fft(y, 1)
                for a in range(16):
                    T[a, pl.ds(h0, 8), ls] = y[a][0]
                    T[a, pl.ds(h0 + 128, 8), ls] = y[a][1]
            return 0
        lax.fori_loop(0, 16, mid, 0)

        def inv(g, _):
            us = [_dot(_bf(cm[24 + g * GA + j]), T[g * GA + j].astype(BF)) for j in range(GA)]
            pv = P[...]
            G = []
            for p in range(4):
                ls = slice(128 * p, 128 * (p + 1))
                re, im = [v[:128, ls] for v in us], [v[128:, ls] for v in us]
                if p == 0:
                    def col(c):
                        return jnp.sum(jnp.where(lane == c, pv, 0.0), axis=1, keepdims=True)
                    re = [jnp.where(lane == 0, col(g * GA + j), re[j]) for j in range(GA)]
                    im = [jnp.where(lane == 0, col(g * GA + j + 16), im[j]) for j in range(GA)]
                v = _dot(jnp.concatenate([jnp.concatenate(re, 0), jnp.concatenate(im, 0)], 1).astype(BF),
                         _bf(cm[4 + p]))
                G.append((v[:, :128], v[:, 128:]))
            s0, s1 = G[0][0] + G[0][1], G[0][0] - G[0][1]
            e = [s0 + G[2][0], s1 - G[2][1], s0 - G[2][0], s1 + G[2][1]]
            a, b = (G[1][0] - G[3][0]) * h, (G[1][1] + G[3][1]) * (-h)
            o = [G[1][0] + G[3][0], b + a, G[3][1] - G[1][1], b - a]
            for t in range(8):
                y = e[t] + o[t] if t < 4 else e[t - 4] - o[t - 4]
                for j in range(GA):
                    rs = pl.ds(g * GA + j, 128, stride=17)
                    x[t, rs, :] = x[t, rs, :] + y[128 * j:128 * (j + 1)]
            return 0
        lax.fori_loop(0, 16 // GA, inv, 0)

    def pair(p, c):
        layer_a()

        @pl.when(p == 0)
        def _():
            for cp in cps[5:]:
                cp.wait()

            def comb(r, c):
                lo = pltpu.bitcast(wrt[r, c].astype(F32), jnp.int32)
                return lax.shift_right_logical(lo, 16) | pltpu.bitcast(wit[r, c].astype(F32), jnp.int32)

            def tr(j, _):
                rs = pl.ds(pl.multiple_of(j * 128, 128), 128)
                wct[...] = comb(slice(0, 512), rs)
                for t, ks in enumerate(PAIRS):
                    wc[rs, 128 * t:128 * (t + 1)] = jnp.concatenate(
                        [wct[pl.ds(k, 64, stride=8), :] for k in ks], 0).T
                return 0
            lax.fori_loop(0, S // 128, tr, 0)
            for m in range(2):
                row = comb(slice(512 * m, 512 * m + 1), slice(None))
                for k in range(16):
                    wsm[16 * m + k:16 * m + k + 1, :] = row[:, 128 * k:128 * (k + 1)]
        layer_b()
        return c
    lax.fori_loop(0, 2, pair, 0)

    outs = []
    for i in range(8):
        rows = pl.ds(i * 256, 256)
        xb[rows, :] = ldb(i * 16, 256).astype(BF)
        c = pltpu.make_async_copy(xb.at[rows], out_hbm.at[rows], sem.at[i])
        c.start()
        outs.append(c)
    for c in outs:
        c.wait()


@jax.jit
def pallas_interleave_layers__sliding_local_dilated__spectral_gfnet__prompt_kernel(
    A_x, A_wqkv, A_wo, B_x, B_w_r, B_w_i):
    consts = _consts()
    I32 = jnp.int32
    anyspec = pl.BlockSpec(memory_space=pl.ANY)
    V = pltpu.VMEM
    out = pl.pallas_call(
        _kernel,
        out_shape=jax.ShapeDtypeStruct((S, D), BF),
        in_specs=[anyspec] * 6 + [pl.BlockSpec(memory_space=V)] * 5,
        out_specs=anyspec,
        scratch_shapes=[
            V((S, D), BF), V((8, S // 16 * 17, 128), F32),
            V((D, 3 * D), BF), V((D // 2, 3 * D), I32), V((D, D), BF), V((D // 2, D), I32),
            V((513, S), BF), V((513, S), BF), V((512, 128), I32), V((S, 512), I32), V((32, 128), I32),
            V(consts[0].shape, I32),
            V((2, 24, BS + 16, 128), F32), V((BS // 2, D), I32), V((2, BS // 2, D), I32),
            V((16, 256, 512), F32), V((128, 128), F32), pltpu.SemaphoreType.DMA((8,))],
        compiler_params=pltpu.CompilerParams(vmem_limit_bytes=110 * 2 ** 20),
    )(A_x.reshape(S, D), A_wqkv, A_wo, B_w_r.T, B_w_i.T, *consts)
    return out.reshape(1, S, D)
```

```python
import numpy as np
import jax
import jax.numpy as jnp
from jax import lax
import jax.experimental.pallas as pl
import jax.experimental.pallas.tpu as pltpu

S, D = 2048, 1024
BS = 256
RC = 64
GA = 4
F32, BF = jnp.float32, jnp.bfloat16


PAIRS = ((0, 4), (1, 7), (2, 6), (3, 5))


def _pack(m):
    u = m.astype(np.float32).astype(BF).view(np.uint16).astype(np.uint32)
    return (u[..., 0::2, :] | (u[..., 1::2, :] << 16)).view(np.int32)


def _consts():
    l = np.arange(128)
    b, j = l[:, None], np.arange(64)[None, :]
    df = np.zeros((4, 256, 256)); di = np.zeros((4, 256, 256))
    for p, (ka, kb) in enumerate(PAIRS):
        ta, tb = (2 * np.pi * b * (k + 8 * j) / 1024 for k in (ka, kb))
        ca, sa, cb, sb = np.cos(ta), np.sin(ta), np.cos(tb), np.sin(tb)
        if p == 0:
            sa[:, 0] = -(-1.0) ** l
            df[p] = np.block([[ca, 0 * ca, -sa, 0 * ca], [0 * ca, cb, 0 * ca, -sb]])
        else:
            df[p] = np.block([[ca, cb, -sa, -sb], [sa, -sb, ca, -cb]])
        di[p] = 2 * df[p].T
    di[0, [0, 128]] /= 2
    grp = (l[:, None] // 4 == l[None, :] // 4) * 1.0
    mf = np.zeros((16, 256, 256)); mi = np.zeros((16, 256, 256))
    for a in range(16):
        t = 2 * np.pi * l[:, None] * (a + 16 * l[None, :]) / 2048
        c, s = np.cos(t), np.sin(t)
        mf[a] = np.block([[c, s], [-s, c]])
        mi[a] = np.block([[c.T, -s.T], [s.T, c.T]]) / (S * D)
    t = 2 * np.pi * l[:, None] * l[None, :] / 128
    f128 = np.concatenate([np.cos(t), -np.sin(t)], 1)
    i128 = f128.T / (S * D)
    r = np.arange(32)
    t = 2 * np.pi * (r[:, None] % 16) * l[None, :] / 2048
    tw = np.concatenate([np.cos(t), -np.sin(t)], 0).astype(np.float32)
    t = 2 * np.pi * (r[:, None] % 16) * (r[None, :] % 16) / 16
    same = r[:, None] // 16 == r[None, :] // 16
    c, s = np.cos(t) * same, np.sin(t) * same
    f16 = np.block([[c, s], [-s, c]])
    return (_pack(np.concatenate([df, di, mf, mi], 0)), _pack(grp), _pack(f128), _pack(i128),
            _pack(np.concatenate([f16, f16.T], 0)), tw)


def _bf(v):
    return pltpu.bitcast(v, BF)


def _i32(v):
    return pltpu.bitcast(v.astype(BF), jnp.int32)


def _dot(a, b):
    return jnp.dot(a, b, preferred_element_type=F32)


def _ln(x):
    m = jnp.mean(x, axis=-1, keepdims=True)
    xc = x - m
    v = jnp.mean(xc * xc, axis=-1, keepdims=True)
    return xc * lax.rsqrt(v + 1e-5)


def _fft(v, sign):
    n = len(v)
    if n == 1:
        return v
    e, o = _fft(v[0::2], sign), _fft(v[1::2], sign)
    out = [None] * n
    for k in range(n // 2):
        er, ei = e[k]
        r, i = o[k]
        if k == 0:
            out[k], out[k + n // 2] = (er + r, ei + i), (er - r, ei - i)
        elif 4 * k == n:
            if sign > 0:
                out[k], out[k + n // 2] = (er - i, ei + r), (er + i, ei - r)
            else:
                out[k], out[k + n // 2] = (er + i, ei - r), (er - i, ei + r)
        else:
            c = float(np.cos(2 * np.pi * k / n)); s = float(sign * np.sin(2 * np.pi * k / n))
            if 8 * k == n or 8 * k == 3 * n:
                h = abs(c)
                if c > 0 and s > 0: tr, ti = (r - i) * h, (r + i) * h
                elif c > 0: tr, ti = (r + i) * h, (i - r) * h
                elif s > 0: tr, ti = (r + i) * (-h), (r - i) * h
                else: tr, ti = (i - r) * h, (r + i) * (-h)
            else:
                tr, ti = r * c - i * s, r * s + i * c
            out[k], out[k + n // 2] = (er + tr, ei + ti), (er - tr, ei - ti)
    return out


def _swap_lanes(w_ref, o_ref, c0):
    def body(r, _):
        rows = pl.ds(pl.multiple_of(r * 128, 128), 128)
        t = [pltpu.bitcast(w_ref[rows, c0 + 128 * u:c0 + 128 * (u + 1)], jnp.int32) for u in range(8)]
        lane = lax.broadcasted_iota(jnp.int32, (64, 128), 1)
        for bit in range(3):
            dist = 4 << bit
            lo = (lane & dist) == 0
            for u in range(8):
                if not u & (1 << bit):
                    a, b = t[u], t[u | (1 << bit)]
                    t[u] = jnp.where(lo, a, pltpu.roll(b, dist, 1))
                    t[u | (1 << bit)] = jnp.where(lo, pltpu.roll(a, 128 - dist, 1), b)
        for u in range(8):
            o_ref[pl.ds(pl.multiple_of(r * 64, 64), 64), c0 + 128 * u:c0 + 128 * (u + 1)] = t[u]
        return 0
    lax.fori_loop(0, D // 128, body, 0)


def _swap_rows(w_ref, o_ref):
    def body(c, _):
        cols = pl.ds(pl.multiple_of(c * 128, 128), 128)
        t = [pltpu.bitcast(w_ref[128 * u:128 * (u + 1), cols], jnp.int32) for u in range(8)]
        row = lax.broadcasted_iota(jnp.int32, (64, 128), 0)
        for bit in range(3):
            dist = 2 << bit
            lo = (row & dist) == 0
            for u in range(8):
                if not u & (1 << bit):
                    a, b = t[u], t[u | (1 << bit)]
                    t[u] = jnp.where(lo, a, pltpu.roll(b, dist, 0))
                    t[u | (1 << bit)] = jnp.where(lo, pltpu.roll(a, 64 - dist, 0), b)
        for u in range(8):
            o_ref[64 * u:64 * (u + 1), cols] = t[u]
        return 0
    lax.fori_loop(0, D // 128, body, 0)


def _kernel(x_hbm, wqkv_hbm, wo_hbm, wr_hbm, wi_hbm, cm_hbm, grp, f128, i128, f16, tw, out_hbm,
            xb, x, wqb, wqkv, wob, wo, wrt, wit, wct, wc, wsm, cm, q, hb, ob, T, P, sem):
    cps = [pltpu.make_async_copy(s, d, sem.at[i]) for i, (s, d) in enumerate(
        [(wqkv_hbm.at[:, pl.ds(j * D, D)], wqb.at[:, pl.ds(j * D, D)]) for j in range(3)]
        + [(x_hbm, xb), (wo_hbm, wob), (wr_hbm, wrt), (wi_hbm, wit), (cm_hbm, cm)])]
    cps[3].start()
    cps[0].start()

    def ldx(rows):
        return jnp.concatenate([x[t, rows, :] for t in range(8)], 1)

    def grp16(m):
        return pl.ds(m * 17, 16)

    def ldb(m0, n):
        return jnp.concatenate([ldx(grp16(m0 + m)) for m in range(n // 16)], 0)

    def stx(rows, v):
        for t in range(8):
            x[t, rows, :] = v[:, 128 * t:128 * (t + 1)]

    def cvt(i, _):
        for m in range(8):
            stx(grp16(i * 8 + m), xb[pl.ds(pl.multiple_of(i * 128 + m * 16, 16), 16), :].astype(F32))
        return 0
    cps[3].wait()
    lax.fori_loop(0, S // 128, cvt, 0)
    for j in range(3):
        cps[j].wait()
        cps[(1, 2, 4)[j]].start()
        _swap_lanes(wqb, wqkv, j * D)
    cps[4].wait()
    for c in cps[5:]:
        c.start()
    _swap_rows(wob, wo)


    def layer_a():
        NC = BS // RC
        CW = 4 * D // NC
        q[0, 8:24, 0:16, :] = jnp.zeros((16, 16, 128), F32)

        def step(i, do_q, do_a, do_o):
            cur = (i + 2) % 2
            nxt = 1 - cur
            if do_q:
                hb[...] = _i32(_ln(ldb((i + 1) * (BS // 16), BS)))
                if do_a:
                    q[nxt, 8:24, 0:16, :] = q[cur, 8:24, BS:BS + 16, :]

            def attn(c, mm):
                r0 = pl.multiple_of(c * RC, RC)
                win = pl.ds(r0, RC + 16)
                r2 = []
                acc = [None] * 8
                for t in range(8):
                    ls = slice(128 * t, 128 * (t + 1))
                    if t % 4 == 0:
                        r2.append(mm(t // 4))
                    qq = q[cur, t, pl.ds(r0 + 16, RC), :]
                    for w in range(8):
                        p = qq * q[cur, 8 + t, pl.ds(r0 + 16 - 2 * w, RC), :]
                        acc[w] = p if t == 0 else acc[w] + p
                lg = _dot(jnp.concatenate(acc, 0).astype(BF), _bf(grp[...]))
                pos = i * BS + r0 + lax.broadcasted_iota(jnp.int32, (RC, 128), 0)
                lg = [jnp.where(pos >= 2 * w, lg[w * RC:(w + 1) * RC] * (32 ** -0.5), -1e9) for w in range(8)]
                m = lg[0]
                for w in range(1, 8):
                    m = jnp.maximum(m, lg[w])
                e = [jnp.exp(l - m) for l in lg]
                tot = e[0]
                for w in range(1, 8):
                    tot = tot + e[w]
                inv = 1.0 / tot
                e = [z * inv for z in e]
                for t in range(8):
                    ls = slice(128 * t, 128 * (t + 1))
                    if t % 4 == 0:
                        r2.append(mm(2 + t // 4))
                    o = e[0] * q[cur, 16 + t, pl.ds(r0 + 16, RC), :]
                    for w in range(1, 8):
                        o = o + e[w] * q[cur, 16 + t, pl.ds(r0 + 16 - 2 * w, RC), :]
                    ob[cur, pl.ds(pl.multiple_of(c * (RC // 2), RC // 2), RC // 2), ls] = _i32(o)

                return r2

            HW = CW // 4

            def both(ca, do, mm):
                if do_a:
                    attn(ca, mm if do else lambda j: None)
                else:
                    for j in range(4):
                        mm(j)
                return 0

            def c1(c, _):
                def mm(j):
                    r = _dot(_bf(hb[...]), _bf(wqkv[:, pl.ds(pl.multiple_of(c * CW + j * HW, HW), HW)]))
                    for t in range(HW // 128):
                        q[nxt, (c * CW + j * HW) // 128 + t, 16:, :] = r[:, 128 * t:128 * (t + 1)]
                return both(c + NC // 4, do_q, mm)

            def c2(c, _):
                def mm(j):
                    r = _dot(_bf(ob[nxt]), _bf(wo[:, pl.ds(pl.multiple_of(c * CW + j * HW, HW), HW)]))
                    for t in range(HW // 128):
                        tt = (c * CW + j * HW) // 128 + t
                        for m in range(BS // 16):
                            rows = grp16((i - 1) * (BS // 16) + m)
                            x[tt, rows, :] = x[tt, rows, :] + r[16 * m:16 * m + 16, 128 * t:128 * (t + 1)]
                return both(c, do_o, mm)
            if do_o or do_a:
                for c in range(NC // 4):
                    c2(c, 0)
            if do_q or do_a:
                for c in range(3 * NC // 4):
                    c1(c, 0)
            return 0
        nb = S // BS
        step(-1, True, False, False)
        step(0, True, True, False)
        lax.fori_loop(1, nb - 1, lambda i, _: step(i, True, True, True), 0)
        step(nb - 1, False, True, True)
        step(nb, False, False, True)

    def layer_b():
        n = GA * 128
        lane = lax.broadcasted_iota(jnp.int32, (128, 128), 1)
        h = float(np.sqrt(0.5))
        P[...] = jnp.zeros((128, 128), F32)

        def fwd(g, _):
            z = _ln(jnp.concatenate(
                [ldx(pl.ds(g * GA + j, 128, stride=17)) for j in range(GA)], 0))
            z = [z[:, 128 * t:128 * (t + 1)] for t in range(8)]
            e = [z[t] + z[t + 4] for t in range(4)]
            o = [z[t] - z[t + 4] for t in range(4)]
            s0, s1 = e[0] + e[2], e[1] + e[3]
            a, b = (o[1] - o[3]) * h, (o[1] + o[3]) * (-h)
            u = [(s0 + s1, s0 - s1), (o[0] + a, b - o[2]),
                 (e[0] - e[2], e[3] - e[1]), (o[0] - a, b + o[2])]
            zz = [_dot(jnp.concatenate(u[p], 1).astype(BF), _bf(cm[p])) for p in range(4)]
            pv = P[...]
            for j in range(GA):
                rs = slice(128 * j, 128 * (j + 1))
                pv = jnp.where(lane == g * GA + j, zz[0][rs, 0:1], pv)
                pv = jnp.where(lane == g * GA + j + 16, zz[0][rs, 128:129], pv)
            P[...] = pv
            zre = jnp.concatenate([v[:, :128] for v in zz], 1).astype(BF)
            zim = jnp.concatenate([v[:, 128:] for v in zz], 1).astype(BF)
            for j in range(GA):
                rs = slice(128 * j, 128 * (j + 1))
                T[g * GA + j] = _dot(_bf(cm[8 + g * GA + j]), jnp.concatenate([zre[rs], zim[rs]], 0))
            return 0
        lax.fori_loop(0, 16 // GA, fwd, 0)

        def wsplit(w):
            return (pltpu.bitcast(w << 16, F32), pltpu.bitcast(w & jnp.int32(-65536), F32))

        g_ = _dot(P[...].T[0:32].astype(BF), _bf(f128[...]))
        gr, gi, tr, ti = g_[:, :128], g_[:, 128:], tw[0:32], tw[32:64]
        g_ = _dot(_bf(f16[0:32]), jnp.concatenate([gr * tr - gi * ti, gr * ti + gi * tr], 0).astype(BF))
        gr, gi = g_[:32], g_[32:]
        ar, ai = wsplit(wsm[...])
        g_ = _dot(_bf(f16[32:64]), jnp.concatenate([gr * ar - gi * ai, gr * ai + gi * ar], 0).astype(BF))
        gr, gi = g_[:32], g_[32:]
        g_ = _dot(jnp.concatenate([gr * tr + gi * ti, gi * tr - gr * ti], 1).astype(BF), _bf(i128[...]))
        P[...] = jnp.concatenate([g_, jnp.zeros((96, 128), F32)], 0).T

        def mid(r, _):
            h0 = pl.multiple_of(r * 8, 8)
            for t in range(4):
                ls = slice(128 * t, 128 * (t + 1))
                v = _fft([(T[a, pl.ds(h0, 8), ls], T[a, pl.ds(h0 + 128, 8), ls]) for a in range(16)], -1)
                y = []
                for k in range(16):
                    a, b = wsplit(wc[pl.ds(h0 + 128 * k, 8), ls])
                    y.append((v[k][0] * a - v[k][1] * b, v[k][0] * b + v[k][1] * a))
                y = _fft(y, 1)
                for a in range(16):
                    T[a, pl.ds(h0, 8), ls] = y[a][0]
                    T[a, pl.ds(h0 + 128, 8), ls] = y[a][1]
            return 0
        lax.fori_loop(0, 16, mid, 0)

        def inv(g, _):
            us = [_dot(_bf(cm[24 + g * GA + j]), T[g * GA + j].astype(BF)) for j in range(GA)]
            pv = P[...]
            G = []
            for p in range(4):
                ls = slice(128 * p, 128 * (p + 1))
                re, im = [v[:128, ls] for v in us], [v[128:, ls] for v in us]
                if p == 0:
                    def col(c):
                        return jnp.sum(jnp.where(lane == c, pv, 0.0), axis=1, keepdims=True)
                    re = [jnp.where(lane == 0, col(g * GA + j), re[j]) for j in range(GA)]
                    im = [jnp.where(lane == 0, col(g * GA + j + 16), im[j]) for j in range(GA)]
                v = _dot(jnp.concatenate([jnp.concatenate(re, 0), jnp.concatenate(im, 0)], 1).astype(BF),
                         _bf(cm[4 + p]))
                G.append((v[:, :128], v[:, 128:]))
            s0, s1 = G[0][0] + G[0][1], G[0][0] - G[0][1]
            e = [s0 + G[2][0], s1 - G[2][1], s0 - G[2][0], s1 + G[2][1]]
            a, b = (G[1][0] - G[3][0]) * h, (G[1][1] + G[3][1]) * (-h)
            o = [G[1][0] + G[3][0], b + a, G[3][1] - G[1][1], b - a]
            for t in range(8):
                y = e[t] + o[t] if t < 4 else e[t - 4] - o[t - 4]
                for j in range(GA):
                    rs = pl.ds(g * GA + j, 128, stride=17)
                    x[t, rs, :] = x[t, rs, :] + y[128 * j:128 * (j + 1)]
            return 0
        lax.fori_loop(0, 16 // GA, inv, 0)

    def pair(p, c):
        layer_a()

        @pl.when(p == 0)
        def _():
            for cp in cps[5:]:
                cp.wait()

            def comb(r, c):
                lo = pltpu.bitcast(wrt[r, c].astype(F32), jnp.int32)
                return lax.shift_right_logical(lo, 16) | pltpu.bitcast(wit[r, c].astype(F32), jnp.int32)

            def tr(j, _):
                rs = pl.ds(pl.multiple_of(j * 128, 128), 128)
                wct[...] = comb(slice(0, 512), rs)
                for t, ks in enumerate(PAIRS):
                    wc[rs, 128 * t:128 * (t + 1)] = jnp.concatenate(
                        [wct[pl.ds(k, 64, stride=8), :] for k in ks], 0).T
                return 0
            lax.fori_loop(0, S // 128, tr, 0)
            for m in range(2):
                row = comb(slice(512 * m, 512 * m + 1), slice(None))
                for k in range(16):
                    wsm[16 * m + k:16 * m + k + 1, :] = row[:, 128 * k:128 * (k + 1)]
        layer_b()
        return c
    lax.fori_loop(0, 2, pair, 0)

    outs = []
    for i in range(8):
        rows = pl.ds(i * 256, 256)
        xb[rows, :] = ldb(i * 16, 256).astype(BF)
        c = pltpu.make_async_copy(xb.at[rows], out_hbm.at[rows], sem.at[i])
        c.start()
        outs.append(c)
    for c in outs:
        c.wait()


@jax.jit
def pallas_interleave_layers__sliding_local_dilated__spectral_gfnet__prompt_kernel(
    A_x, A_wqkv, A_wo, B_x, B_w_r, B_w_i):
    consts = _consts()
    I32 = jnp.int32
    anyspec = pl.BlockSpec(memory_space=pl.ANY)
    V = pltpu.VMEM
    out = pl.pallas_call(
        _kernel,
        out_shape=jax.ShapeDtypeStruct((S, D), BF),
        in_specs=[anyspec] * 6 + [pl.BlockSpec(memory_space=V)] * 5,
        out_specs=anyspec,
        scratch_shapes=[
            V((S, D), BF), V((8, S // 16 * 17, 128), F32),
            V((D, 3 * D), BF), V((D // 2, 3 * D), I32), V((D, D), BF), V((D // 2, D), I32),
            V((513, S), BF), V((513, S), BF), V((512, 128), I32), V((S, 512), I32), V((32, 128), I32),
            V(consts[0].shape, I32),
            V((2, 24, BS + 16, 128), F32), V((BS // 2, D), I32), V((2, BS // 2, D), I32),
            V((16, 256, 512), F32), V((128, 128), F32), pltpu.SemaphoreType.DMA((8,))],
        compiler_params=pltpu.CompilerParams(vmem_limit_bytes=110 * 2 ** 20),
    )(A_x.reshape(S, D), A_wqkv, A_wo, B_w_r.T, B_w_i.T, *consts)
    return out.reshape(1, S, D)
```
